```python
import os as _os
_os.environ.setdefault("JAX_PLATFORMS", "cpu")
import jax
import jax.numpy as jnp

def _softmax(x, axis=-1):
    return jax.nn.softmax(x, axis=axis)
def _gelu(x):
    return jax.nn.gelu(x, approximate=True)
def _silu(x):
    return jax.nn.silu(x)
def _sigmoid(x):
    return jax.nn.sigmoid(x)
def _layernorm(x, axis=-1, eps=1e-5):
    m = jnp.mean(x, axis=axis, keepdims=True)
    v = jnp.var(x, axis=axis, keepdims=True)
    return (x - m) / jnp.sqrt(v + eps)
def _scatter_add(tgt, idx, src, axis=0):
    return tgt.at[idx].add(src)
def _segment_sum(src, seg, n):
    return jax.ops.segment_sum(src, seg, n)
class _Rng:
    def __init__(self, key):
        self._k = key
    def _next(self):
        self._k, sub = jax.random.split(self._k)
        return sub
    def normal(self, shape):
        return jax.random.normal(self._next(), shape, dtype=jnp.bfloat16)
    def randint(self, lo, hi, shape):
        return jax.random.randint(self._next(), shape, lo, hi, dtype=jnp.int32)
    def uniform(self, shape, lo=0.0, hi=1.0):
        return jax.random.uniform(self._next(), shape, jnp.bfloat16, lo, hi)
    def permutation(self, n):
        return jax.random.permutation(self._next(), n)


kernel_name = 'concat_heads__mha_block_cached__mha_block_cached__near_ridge'

def setup_inputs():
    _rng = _Rng(jax.random.key(int.from_bytes(__import__("os").urandom(4), "little")))
    _w = (lambda a: (lambda t: t.astype(jnp.bfloat16) if jnp.issubdtype(t.dtype, jnp.floating) else t)(jnp.asarray(a)))
    def _A_setup():
        B, Sq, D = 16, 32, 1024
        H, Sk, Dh = 32, 32, 128
        return {
            "x": _w((lambda *s: _rng.normal(s) * 0.8)(B, Sq, D)),
            "k_cache": _w((lambda *s: _rng.normal(s) * 0.8)(B, H, Sk, Dh)),
            "v_cache": _w((lambda *s: _rng.normal(s) * 0.05)(B, H, Sk, Dh)),
            "wq": _w((lambda *s: _rng.normal(s) * 0.8)(D, H * Dh) * (D ** -0.5)),
            "wo": _w((lambda *s: _rng.normal(s) * 0.05)(H * Dh, D) * ((H * Dh) ** -0.5)),
        }
    _A_in = _A_setup()

    def _B_setup():
        B, Sq, D = 16, 32, 1024
        H, Sk, Dh = 32, 32, 128
        return {
            "x": _w((lambda *s: _rng.normal(s) * 0.8)(B, Sq, D)),
            "k_cache": _w((lambda *s: _rng.normal(s) * 0.8)(B, H, Sk, Dh)),
            "v_cache": _w((lambda *s: _rng.normal(s) * 0.05)(B, H, Sk, Dh)),
            "wq": _w((lambda *s: _rng.normal(s) * 0.8)(D, H * Dh) * (D ** -0.5)),
            "wo": _w((lambda *s: _rng.normal(s) * 0.05)(H * Dh, D) * ((H * Dh) ** -0.5)),
        }
    _B_in = _B_setup()

    return {
        "A_x": _A_in["x"],
        "A_k_cache": _A_in["k_cache"],
        "A_v_cache": _A_in["v_cache"],
        "A_wq": _A_in["wq"],
        "A_wo": _A_in["wo"],
        "B_x": _B_in["x"],
        "B_k_cache": _B_in["k_cache"],
        "B_v_cache": _B_in["v_cache"],
        "B_wq": _B_in["wq"],
        "B_wo": _B_in["wo"],
    }

def reference(A_x, A_k_cache, A_v_cache, A_wq, A_wo, B_x, B_k_cache, B_v_cache, B_wq, B_wo):
    def _A_ref(x, k_cache, v_cache, wq, wo):
        B, Sq, D = x.shape
        H, Dh = 32, 128
        q = (lambda x, *d: x.transpose(*d))((x @ wq).reshape(B, Sq, H, Dh), 0, 2, 1, 3)
        scores = jnp.einsum("bhqd,bhkd->bhqk", q, k_cache) * (Dh ** -0.5)
        p = _softmax(scores, axis=-1)
        o = jnp.einsum("bhqk,bhkd->bhqd", p, v_cache)
        return (lambda x, *d: x.transpose(*d))(o, 0, 2, 1, 3).reshape(B, Sq, H * Dh) @ wo

    def _B_ref(x, k_cache, v_cache, wq, wo):
        B, Sq, D = x.shape
        H, Dh = 32, 128
        q = (lambda x, *d: x.transpose(*d))((x @ wq).reshape(B, Sq, H, Dh), 0, 2, 1, 3)
        scores = jnp.einsum("bhqd,bhkd->bhqk", q, k_cache) * (Dh ** -0.5)
        p = _softmax(scores, axis=-1)
        o = jnp.einsum("bhqk,bhkd->bhqd", p, v_cache)
        return (lambda x, *d: x.transpose(*d))(o, 0, 2, 1, 3).reshape(B, Sq, H * Dh) @ wo

    a = _A_ref(A_x, A_k_cache, A_v_cache, A_wq, A_wo)
    b = _B_ref(B_x, B_k_cache, B_v_cache, B_wq, B_wo)
    return jnp.concatenate([a, b], axis=-1)
```

```python
import functools
import jax
import jax.numpy as jnp
from jax import lax
import jax.experimental.pallas as pl
import jax.experimental.pallas.tpu as pltpu

B, SQ, D = 16, 32, 1024
H, SK, DH = 32, 32, 128
M = B * SQ
GB = 4
NG = B // GB
LOG2E = 1.4426950408889634
F32 = jnp.float32
BF16 = jnp.bfloat16

START = [
    ([("x", 0, 0), ("q", 0, 1)], "QP0"),
    ([("q", 1, 3)], "QP1 QP2"),
    ([("q", 3, 7)], "QP3 QP4 QP5 QP6"),
    ([("k", 0, 4), ("q", 7, 8), ("v", 0, 4), ("o", 0, 3)], "QK0 QK1 QP7 PV0 PV1 QK2 QK3 OP0 PV2 PV3 OP1 OP2"),
    ([("k", 4, 8), ("v", 4, 8), ("o", 3, 8)], "QK4 QK5 OP3 PV4 PV5 QK6 QK7 OP4 PV6 PV7 OP5 OP6 OP7"),
]
S = 8
U1, N1 = 4, 2
U2, N2 = 8, 6
ORD1 = "QP0 QP1 QK0 QP2 PV0 QK1 QP3 PV1 QK2 OP0 PV2 QK3 OP1 PV3 OP2 OP3"
ORD2 = ("QP0 QP1 QK0 QP2 PV0 QK1 QP3 PV1 QK2 QP4 PV2 QK3 QP5 PV3 QK4 QP6 PV4 QK5 QP7 PV5 "
        "QK6 OP0 PV6 QK7 OP1 PV7 OP2 OP3 OP4 OP5 FF6")
assert S + U1 * N1 + U2 * N2 == 2 * H


def parse(s):
    return [(t[:2], int(t[2:])) for t in s.split()]


def impl(A_x, A_k, A_v, A_wq, A_wo, B_x, B_k, B_v, B_wq, B_wo, nf=8, ord2=ORD2):
    c = (DH ** -0.5) * LOG2E
    n_start_dma = sum(len(d) for d, _ in START)
    SEM1 = n_start_dma
    SEM2 = SEM1 + 4 * N1
    SEMX = SEM2 + 4 * N2
    SEMO = SEMX + 1
    NSEM = SEMO + 2 * nf
    RF = M // nf

    def kernel(xa, ka, va, wqa, woa, xb, kb, vb, wqb, wob, out_hbm,
               x_buf, wq_s, wq_1, wq_2, wo_buf, k_buf, v_buf, acc, out_buf, q_buf, o_buf, sems):
        srcs = ((xa, ka, va, wqa, woa), (xb, kb, vb, wqb, wob))

        def dma(kind, br, lo, hi, wq_dst, sem):
            x, k, v, wq, wo = srcs[br]
            n = hi - lo
            if kind == "x":
                return pltpu.make_async_copy(x, x_buf.at[br], sem)
            if kind == "q":
                return pltpu.make_async_copy(wq.at[:, pl.ds(lo * DH, n * DH)], wq_dst, sem)
            if kind == "k":
                return pltpu.make_async_copy(k.at[:, pl.ds(lo, n)], k_buf.at[br, :, pl.ds(lo, n)], sem)
            if kind == "v":
                return pltpu.make_async_copy(v.at[:, pl.ds(lo, n)], v_buf.at[br, :, pl.ds(lo, n)], sem)
            return pltpu.make_async_copy(wo.at[pl.ds(lo * DH, n * DH), :], wo_buf.at[br, pl.ds(lo * DH, n * DH), :], sem)

        def out_dma(br, t):
            return pltpu.make_async_copy(
                out_buf.at[br, t], out_hbm.at[pl.ds(t * RF, RF), pl.ds(pl.multiple_of(br * D, D), D)],
                sems.at[SEMO + br * nf + t])

        start_cps = []
        si = 0
        for dl, _ in START:
            seg = []
            for kind, lo, hi in dl:
                seg.append(dma(kind, 0, lo, hi, wq_s.at[:, pl.ds(lo * DH, (hi - lo) * DH)], sems.at[si]))
                si += 1
            start_cps.append(seg)
        for seg in start_cps:
            for cp in seg:
                cp.start()
        for i in range(N1):
            lo = S + i * U1
            for j, kind in enumerate("qkvo"):
                dma(kind, 0, lo, lo + U1, wq_1.at[i], sems.at[SEM1 + 4 * i + j]).start()
        for i in range(N2):
            g = S + N1 * U1 + i * U2
            br, lo = g // H, g % H
            if lo == 0:
                dma("x", br, 0, 0, None, sems.at[SEMX]).start()
            for j, kind in enumerate("qkvo"):
                dma(kind, br, lo, lo + U2, wq_2.at[i], sems.at[SEM2 + 4 * i + j]).start()
        acc[1] = jnp.zeros((M, D), F32)

        row = lax.broadcasted_iota(jnp.int32, (128, 128), 0) // SQ
        col = lax.broadcasted_iota(jnp.int32, (128, 128), 1) // SK
        mask = row == col

        def run(order, br, h0, wq_ref, ps, first=False, last=None):
            for op, j in order:
                if op == "QP":
                    q = jnp.dot(x_buf[br], wq_ref[:, j * DH:(j + 1) * DH], preferred_element_type=F32)
                    q_buf[j] = q.astype(BF16)
                elif op == "QK":
                    for t in range(NG):
                        q = q_buf[j, t * 128:(t + 1) * 128, :]
                        k = k_buf[br, t * GB:(t + 1) * GB, h0 + j].reshape(128, DH)
                        s = lax.dot_general(q, k, (((1,), (1,)), ((), ())), preferred_element_type=F32)
                        s = jnp.where(mask, s, -jnp.inf)
                        m = jnp.max(s, axis=-1, keepdims=True)
                        p = jnp.exp2((s - m) * c)
                        l = jnp.sum(p, axis=-1, keepdims=True)
                        r = pl.reciprocal(l, approx=False, full_range=False)
                        ps[(j, t)] = (p * r).astype(BF16)
                elif op == "PV":
                    for t in range(NG):
                        v = v_buf[br, t * GB:(t + 1) * GB, h0 + j].reshape(128, DH)
                        o = jnp.dot(ps.pop((j, t)), v, preferred_element_type=F32)
                        o_buf[t * 128:(t + 1) * 128, j * DH:(j + 1) * DH] = o.astype(BF16)
                elif op == "OP":
                    w = wo_buf[br, pl.ds(pl.multiple_of((h0 + j) * DH, DH), DH), :]
                    r = jnp.dot(o_buf[:, j * DH:(j + 1) * DH], w, preferred_element_type=F32)
                    if first and j == 0:
                        acc[br] = r
                    else:
                        acc[br] = acc[br] + r
                elif op == "FF":
                    nh = U2 - j
                    for t in range(nf):
                        w = wo_buf[br, pl.ds(pl.multiple_of((h0 + j) * DH, DH), nh * DH), :]
                        r = jnp.dot(o_buf[t * RF:(t + 1) * RF, j * DH:U2 * DH], w, preferred_element_type=F32)
                        r = acc[br, t * RF:(t + 1) * RF, :] + r
                        acc[br, t * RF:(t + 1) * RF, :] = r
                        out_buf[br, t] = r.astype(BF16)

                        @pl.when(last)
                        def _():
                            out_dma(br, t).start()

        def wait4(br, h0, n, wq_ref, sem0):
            hs = pl.ds(h0, n)
            rs = pl.ds(pl.multiple_of(h0 * DH, DH), n * DH)
            for j, r in enumerate((wq_ref, k_buf.at[br, :, hs], v_buf.at[br, :, hs], wo_buf.at[br, rs, :])):
                pltpu.make_async_copy(r, r, sems.at[sem0 + j]).wait()

        ps = {}
        for seg, (_, ops) in zip(start_cps, START):
            for cp in seg:
                cp.wait()
            run(parse(ops), 0, 0, wq_s, ps, first=True)

        def body1(i, carry):
            h0 = S + i * U1
            wait4(0, h0, U1, wq_1.at[i], SEM1 + 4 * i)
            run(parse(ORD1), 0, h0, wq_1.at[i], {})
            return carry

        lax.fori_loop(0, N1, body1, 0)

        def body2(i, carry):
            g = S + N1 * U1 + i * U2
            br = g // H
            h0 = g % H

            @pl.when(h0 == 0)
            def _():
                pltpu.make_async_copy(x_buf.at[1], x_buf.at[1], sems.at[SEMX]).wait()

            wait4(br, h0, U2, wq_2.at[i], SEM2 + 4 * i)
            run(parse(ord2), br, h0, wq_2.at[i], {}, last=(h0 == H - U2))
            return carry

        lax.fori_loop(0, N2, body2, 0)
        for br in range(2):
            for t in range(nf):
                out_dma(br, t).wait()

    any_spec = pl.BlockSpec(memory_space=pl.ANY)
    out = pl.pallas_call(
        kernel,
        in_specs=[any_spec] * 10,
        out_specs=any_spec,
        out_shape=jax.ShapeDtypeStruct((M, 2 * D), BF16),
        scratch_shapes=[
            pltpu.VMEM((2, M, D), BF16),
            pltpu.VMEM((D, S * DH), BF16),
            pltpu.VMEM((N1, D, U1 * DH), BF16),
            pltpu.VMEM((N2, D, U2 * DH), BF16),
            pltpu.VMEM((2, H * DH, D), BF16),
            pltpu.VMEM((2, B, H, SK, DH), BF16),
            pltpu.VMEM((2, B, H, SK, DH), BF16),
            pltpu.VMEM((2, M, D), F32),
            pltpu.VMEM((2, nf, RF, D), BF16),
            pltpu.VMEM((8, M, DH), BF16),
            pltpu.VMEM((M, 8 * DH), BF16),
            pltpu.SemaphoreType.DMA((NSEM,)),
        ],
        compiler_params=pltpu.CompilerParams(
            vmem_limit_bytes=100 * 1024 * 1024, disable_bounds_checks=True, disable_semaphore_checks=True),
    )(A_x.reshape(M, D), A_k, A_v, A_wq, A_wo, B_x.reshape(M, D), B_k, B_v, B_wq, B_wo)
    return out.reshape(B, SQ, 2 * D)


@jax.jit
def pallas_concat_heads__mha_block_cached__mha_block_cached__near_ridge_kernel(
    A_x: jax.Array,
    A_k_cache: jax.Array,
    A_v_cache: jax.Array,
    A_wq: jax.Array,
    A_wo: jax.Array,
    B_x: jax.Array,
    B_k_cache: jax.Array,
    B_v_cache: jax.Array,
    B_wq: jax.Array,
    B_wo: jax.Array,
):
    return impl(A_x, A_k_cache, A_v_cache, A_wq, A_wo, B_x, B_k_cache, B_v_cache, B_wq, B_wo)
```

```python
import jax
import jax.numpy as jnp
from jax import lax
import jax.experimental.pallas as pl
import jax.experimental.pallas.tpu as pltpu

B, SQ, D = 16, 32, 1024
H, SK, DH = 32, 32, 128
M = B * SQ
GB = 4
NG = B // GB
KT = D // 128
LOG2E = 1.4426950408889634
F32 = jnp.float32
BF16 = jnp.bfloat16
PAD = 128

START = [
    "x0-1 q0-8:0-1 | QS0-8:0-1",
    "q8-16:0-1 x1-2 q0-4:1-2 | QS8-16:0-1 QS0-4:1-2",
    "q4-16:1-2 x2-3 q0-8:2-3 | QS4-16:1-2 QS0-8:2-3",
    "q8-16:2-3 x3-5 q0-16:3-4 q0-8:4-5 | QS8-16:2-4 QS0-8:3-5",
    "q8-16:4-5 x5-8 q0-16:5-8 | QS8-16:4-8 QS0-8:5-8",
]
S = 16
U1 = 8
N1 = (H - S) // U1
U2 = 8
N2 = H // U2
U3 = 16
N3 = H // U3
L3 = 6
P2 = (H - N3 * L3) // N2
NFF = 3
ROWS = (128, 128, 96, 64, 48, 48)
assert N1 == 2 and N2 == 2 * N3 and sum(ROWS) == M


def _rng(s):
    a, b = s.split("-")
    return int(a), int(b)


def _parse_ops(s):
    out = []
    for t in s.split():
        if t[:2] == "QS":
            h, k = t[2:].split(":")
            out.append(("QS", _rng(h) + _rng(k)))
        else:
            out.append((t[:2], int(t[2:])))
    return out


def _parse_dmas(s):
    out = []
    for t in s.split():
        body = t[1:].split(":")
        out.append((t[0], _rng(body[0]), _rng(body[1]) if len(body) > 1 else (0, KT)))
    return out


def _chain(n, covers):
    o = ["QP0", "QK0"]
    for j in range(n):
        o += [covers[j], f"MM{j}" if j + 1 < n else f"PV{j}"]
    return _parse_ops(" ".join(o + covers[n:]))


_START = [(_parse_dmas(s.split("|")[0]), _parse_ops(s.split("|")[1])) for s in START]
_ORD1 = _parse_ops("ZZ0 " + " ".join(f"QP{j}" for j in range(U1)))
_ORD2 = _chain(U2, [f"QP{j}" for j in range(1, P2)] + [f"OP{j}" for j in range(U2 - 1)] + [f"OW{U2 - 1}"])
_ORD3 = _chain(U3, [f"QP{j}" for j in range(1, L3)] + [f"OP{j}" for j in range(U3 - NFF)] + [f"FF{U3 - NFF}"])
_ROFF = [sum(ROWS[:t]) for t in range(len(ROWS))]

SEM1 = sum(len(d) for d, _ in _START)
SEMX = SEM1 + N1
SEM2 = SEMX + 1
SEM3 = SEM2 + 4 * N2
SEMA = SEM3 + 4 * N3
SEMO = SEMA + 1
NSEM = SEMO + len(ROWS)


def _kernel(xa, ka, va, wqa, woa, xb, kb, vb, wqb, wob, out_hbm,
            x_buf, wq_s, wq_1, wq_2, wq_3, wo_buf, k_buf, v_buf, acc, out_a, out_b,
            q_a, q_b, q_l, o_buf, qa_buf, sems):
    srcs = ((xa, ka, va, wqa, woa), (xb, kb, vb, wqb, wob))
    c = (DH ** -0.5) * LOG2E

    def dma(kind, br, hr, kr, wq_dst, sem):
        x, k, v, wq, wo = srcs[br]
        lo, n = hr[0], hr[1] - hr[0]
        if kind == "x":
            cs = pl.ds(lo * 128, n * 128)
            return pltpu.make_async_copy(x.at[:, cs], x_buf.at[br, :, cs], sem)
        if kind == "q":
            rs = pl.ds(kr[0] * 128, (kr[1] - kr[0]) * 128)
            return pltpu.make_async_copy(wq.at[rs, pl.ds(lo * DH, n * DH)], wq_dst.at[rs, :], sem)
        if kind == "k":
            return pltpu.make_async_copy(k.at[:, pl.ds(lo, n)], k_buf.at[br, :, pl.ds(lo, n)], sem)
        if kind == "v":
            return pltpu.make_async_copy(v.at[:, pl.ds(lo, n)], v_buf.at[br, :, pl.ds(lo, n)], sem)
        rs = pl.ds(lo * DH, n * DH)
        return pltpu.make_async_copy(wo.at[rs, :], wo_buf.at[br, rs, :], sem)

    def outa_dma():
        return pltpu.make_async_copy(out_a, out_hbm.at[:, pl.ds(0, D)], sems.at[SEMA])

    def outb_dma(t):
        rs = pl.ds(_ROFF[t], ROWS[t])
        return pltpu.make_async_copy(out_b.at[rs, :], out_hbm.at[rs, pl.ds(D, D)], sems.at[SEMO + t])

    def start_copies():
        cps, si = [], 0
        for dl, _ in _START:
            seg = []
            for kind, hr, kr in dl:
                dst = wq_s.at[:, pl.ds(hr[0] * DH, (hr[1] - hr[0]) * DH)] if kind == "q" else None
                seg.append(dma(kind, 0, hr, kr, dst, sems.at[si]))
                si += 1
            cps.append(seg)
        return cps

    for seg in start_copies():
        for cp in seg:
            cp.start()
    for i in range(N1):
        lo = S + i * U1
        dma("q", 0, (lo, lo + U1), (0, KT), wq_1.at[i, :, pl.ds(0, U1 * DH)], sems.at[SEM1 + i]).start()
    dma("x", 1, (0, KT), None, None, sems.at[SEMX]).start()
    for i in range(N2):
        lo = i * P2 + (i // 2) * L3
        dma("q", 1, (lo, lo + P2), (0, KT), wq_2.at[i], sems.at[SEM2 + 4 * i]).start()
        for j, kind in enumerate("kvo"):
            dma(kind, 0, (i * U2, (i + 1) * U2), None, None, sems.at[SEM2 + 4 * i + 1 + j]).start()
    for i in range(N3):
        lo, hi = i * U3, (i + 1) * U3
        dma("q", 1, (hi - L3, hi), (0, KT), wq_3.at[i, :, pl.ds(0, L3 * DH)], sems.at[SEM3 + 4 * i]).start()
        for j, kind in enumerate("kvo"):
            dma(kind, 1, (lo, hi), None, None, sems.at[SEM3 + 4 * i + 1 + j]).start()

    def run(order, it, pbr, ph0, wq_ref, abr, ah0, last=None):
        phase3 = last is not None
        q_dst = (q_a, q_b)[pbr]
        q_src = (q_a, q_b)[abr] if abr is not None else None
        colb = lax.broadcasted_iota(jnp.int32, (SQ, 128), 1) // SK
        colh = lax.broadcasted_iota(jnp.int32, (SQ // 2, 128), 1) // SK
        zero = jnp.zeros((SQ // 2, 128), jnp.uint32)
        ps = {}

        def u32(a):
            return pltpu.bitcast(a, jnp.uint32)

        def sel(i, a, b):
            return pltpu.bitcast(jnp.where(colh == i, u32(a), u32(b)), BF16)

        def keep(i, a):
            return pltpu.bitcast(jnp.where(colh != i, zero, u32(a)), BF16)

        def drop(i, a):
            return pltpu.bitcast(jnp.where(colh == i, zero, u32(a)), BF16)

        def blk(a, i):
            return a[i * SQ:(i + 1) * SQ, :]

        def compact(parts):
            r = parts[GB - 1]
            for i in range(GB - 2, -1, -1):
                r = jnp.where(colb == i, parts[i], r)
            return r

        def q_tile(j, t):
            if phase3 and j >= U3 - L3:
                return q_l[j - (U3 - L3), t * 128:(t + 1) * 128, :]
            return q_src[ah0 + j, t * 128:(t + 1) * 128, :]

        def k_tile(j, t):
            return k_buf[abr, t * GB:(t + 1) * GB, ah0 + j].reshape(128, DH)

        def v_tile(j, t):
            return v_buf[abr, t * GB:(t + 1) * GB, ah0 + j].reshape(128, DH)

        def wo_rows(j, n):
            return wo_buf[abr, pl.ds(pl.multiple_of((ah0 + j) * DH, DH), n * DH), :]

        def softmax(sc):
            mc = compact([jnp.max(jnp.where(colb == i, sc, -jnp.inf), axis=-1, keepdims=True)
                          for i in range(GB)])
            e = jnp.exp2((sc - mc) * c)
            lc = compact([jnp.sum(jnp.where(colb == i, e, 0.0), axis=-1, keepdims=True)
                          for i in range(GB)])
            return (e * pl.reciprocal(lc, approx=False, full_range=False)).astype(BF16)

        for op, j in order:
            if op == "QP":
                q = jnp.dot(x_buf[pbr], wq_ref[:, j * DH:(j + 1) * DH], preferred_element_type=F32)
                if phase3:
                    q_l[j] = q.astype(BF16)
                else:
                    q_dst[ph0 + j] = q.astype(BF16)
            elif op == "QS":
                ja, jb, k0, k1 = j
                q = jnp.dot(x_buf[pbr, :, k0 * 128:k1 * 128], wq_ref[k0 * 128:k1 * 128, ja * DH:jb * DH],
                            preferred_element_type=F32)
                for jj in range(ja, jb):
                    qq = q[:, (jj - ja) * DH:(jj - ja + 1) * DH]
                    if k0 > 0:
                        qq = qa_buf[jj] + qq
                    if k1 == KT:
                        q_dst[jj] = qq.astype(BF16)
                    else:
                        qa_buf[jj] = qq
            elif op == "ZZ":
                acc[it] = jnp.zeros((M, D), F32)
            elif op == "QK":
                for t in range(NG):
                    s = lax.dot_general(q_tile(j, t), k_tile(j, t), (((1,), (1,)), ((), ())),
                                        preferred_element_type=F32)
                    ps[t] = softmax(compact([blk(s, i) for i in range(GB)]))
            elif op == "MM":
                for t in range(NG):
                    kt = k_tile(j + 1, t).T
                    v = v_tile(j, t)
                    q = q_tile(j + 1, t)
                    pc = ps[t]
                    qc = blk(q, GB - 1)
                    for i in range(GB - 2, -1, -1):
                        qc = sel(i, blk(q, i), qc)
                    wdk = jnp.concatenate([keep(i, blk(kt, i)) for i in range(GB)], axis=0)
                    wdv = jnp.concatenate([keep(i, blk(v, i)) for i in range(GB)], axis=0)
                    tail_s = jnp.dot(qc, wdk, preferred_element_type=F32)
                    tail_o = jnp.dot(pc, wdv, preferred_element_type=F32)
                    mains = []
                    for i in range(GB):
                        w = jnp.concatenate(
                            [drop(i, blk(v, i)) if r == i else keep(i, blk(kt, r)) for r in range(GB)], axis=0)
                        mains.append(jnp.dot(sel(i, pc, blk(q, i)), w, preferred_element_type=F32))
                    ps[t] = softmax(compact(mains) + tail_s)
                    o = jnp.concatenate([jnp.where(colb == i, tail_o, mains[i]) for i in range(GB)], axis=0)
                    o_buf[t * 128:(t + 1) * 128, j * DH:(j + 1) * DH] = o.astype(BF16)
            elif op == "PV":
                for t in range(NG):
                    p = jnp.concatenate([keep(i, ps[t]) for i in range(GB)], axis=0)
                    o = jnp.dot(p, v_tile(j, t), preferred_element_type=F32)
                    o_buf[t * 128:(t + 1) * 128, j * DH:(j + 1) * DH] = o.astype(BF16)
            elif op in ("OP", "OW"):
                r = acc[abr] + jnp.dot(o_buf[:, j * DH:(j + 1) * DH], wo_rows(j, 1), preferred_element_type=F32)
                acc[abr] = r
                if op == "OW":
                    out_a[...] = r.astype(BF16)
            else:
                for t in range(len(ROWS)):
                    rs = slice(_ROFF[t], _ROFF[t] + ROWS[t])
                    r = acc[abr, rs, :] + jnp.dot(o_buf[rs, j * DH:U3 * DH], wo_rows(j, U3 - j),
                                                  preferred_element_type=F32)
                    acc[abr, rs, :] = r
                    out_b[rs, :] = r.astype(BF16)

                    @pl.when(last)
                    def _():
                        outb_dma(t).start()

    def wait(r, sem):
        pltpu.make_async_copy(r, r, sems.at[sem]).wait()

    def wait_kvo(br, h0, n, sem0):
        hs = pl.ds(h0, n)
        rs = pl.ds(pl.multiple_of(h0 * DH, DH), n * DH)
        for j, r in enumerate((k_buf.at[br, :, hs], v_buf.at[br, :, hs], wo_buf.at[br, rs, :])):
            wait(r, sem0 + j)

    def body1(i, carry):
        wait(wq_1.at[i, :, pl.ds(0, U1 * DH)], SEM1 + i)
        run(_ORD1, i, 0, S + i * U1, wq_1.at[i], None, None)
        return carry

    def body2(i, carry):
        wait(wq_2.at[i], SEM2 + 4 * i)
        wait_kvo(0, i * U2, U2, SEM2 + 4 * i + 1)
        run(_ORD2, i, 1, i * P2 + lax.shift_right_logical(i, 1) * L3, wq_2.at[i], 0, i * U2)
        return carry

    def body3(i, carry):
        wait(wq_3.at[i, :, pl.ds(0, L3 * DH)], SEM3 + 4 * i)
        wait_kvo(1, i * U3, U3, SEM3 + 4 * i + 1)
        run(_ORD3, i, 1, None, wq_3.at[i], 1, i * U3, last=(i == N3 - 1))
        return carry

    def phase(ph, carry):
        @pl.when(ph == 0)
        def _():
            for seg, (_, ops) in zip(start_copies(), _START):
                for cp in seg:
                    cp.wait()
                run(ops, None, 0, 0, wq_s, None, None)
            lax.fori_loop(0, N1, body1, 0)
            wait(x_buf.at[1], SEMX)
            lax.fori_loop(0, N2, body2, 0)
            outa_dma().start()

        @pl.when(ph == 1)
        def _():
            lax.fori_loop(0, N3, body3, 0)
        return carry

    lax.fori_loop(0, 2, phase, 0)
    outa_dma().wait()
    for t in range(len(ROWS)):
        outb_dma(t).wait()


@jax.jit
def pallas_concat_heads__mha_block_cached__mha_block_cached__near_ridge_kernel(
    A_x: jax.Array,
    A_k_cache: jax.Array,
    A_v_cache: jax.Array,
    A_wq: jax.Array,
    A_wo: jax.Array,
    B_x: jax.Array,
    B_k_cache: jax.Array,
    B_v_cache: jax.Array,
    B_wq: jax.Array,
    B_wo: jax.Array,
):
    any_spec = pl.BlockSpec(memory_space=pl.ANY)
    out = pl.pallas_call(
        _kernel,
        in_specs=[any_spec] * 10,
        out_specs=any_spec,
        out_shape=jax.ShapeDtypeStruct((M, 2 * D), BF16),
        scratch_shapes=[
            pltpu.VMEM((2, M, D), BF16),
            pltpu.VMEM((D, S * DH + PAD), BF16),
            pltpu.VMEM((N1, D, U1 * DH + PAD), BF16),
            pltpu.VMEM((N2, D, P2 * DH), BF16),
            pltpu.VMEM((N3, D, L3 * DH + PAD), BF16),
            pltpu.VMEM((2, H * DH, D), BF16),
            pltpu.VMEM((2, B, H, SK, DH), BF16),
            pltpu.VMEM((2, B, H, SK, DH), BF16),
            pltpu.VMEM((2, M, D), F32),
            pltpu.VMEM((M, D), BF16),
            pltpu.VMEM((M, D), BF16),
            pltpu.VMEM((H, M, DH), BF16),
            pltpu.VMEM((H, M, DH), BF16),
            pltpu.VMEM((L3, M, DH), BF16),
            pltpu.VMEM((M, U3 * DH), BF16),
            pltpu.VMEM((S, M, DH), F32),
            pltpu.SemaphoreType.DMA((NSEM,)),
        ],
        compiler_params=pltpu.CompilerParams(
            vmem_limit_bytes=110 * 1024 * 1024,
            disable_bounds_checks=True,
            disable_semaphore_checks=True,
        ),
    )(A_x.reshape(M, D), A_k_cache, A_v_cache, A_wq, A_wo,
      B_x.reshape(M, D), B_k_cache, B_v_cache, B_wq, B_wo)
    return out.reshape(B, SQ, 2 * D)
```

```python
import jax
import jax.numpy as jnp
from jax import lax
import jax.experimental.pallas as pl
import jax.experimental.pallas.tpu as pltpu

B, SQ, D = 16, 32, 1024
H, SK, DH = 32, 32, 128
M = B * SQ
GB = 4
NG = B // GB
KT = D // 128
LOG2E = 1.4426950408889634
F32 = jnp.float32
BF16 = jnp.bfloat16
U32 = jnp.uint32
PAD = 128

START = [
    "x0-1 q0-8:0-1 | QS0-8:0-1",
    "q8-16:0-1 x1-2 q0-4:1-2 | QS8-16:0-1 QS0-4:1-2",
    "q4-16:1-2 x2-3 q0-8:2-3 | QS4-16:1-2 QS0-8:2-3",
    "q8-16:2-3 x3-5 q0-16:3-4 q0-12:4-5 | QS8-12:2-5 QS12-16:2-4 QS0-8:3-5",
    "q12-16:4-5 x5-8 q0-16:5-8 k0-1 | QS0-8:5-8 QS8-12:5-8 QK0 QS12-16:4-8",
]
S = 16
U1 = 8
N1 = (H - S) // U1
U2 = 8
N2 = H // U2
U3 = 16
N3 = H // U3
L3 = 4
P2 = (H - N3 * L3) // N2
NFF = 3
ROWS = (128, 128, 96, 64, 48, 48)
W2 = D + P2 * DH + (PAD if P2 % 2 == 0 else 0)
W3 = D + (L3 // 2) * DH + (PAD if (L3 // 2) % 2 == 0 else 0)
assert N1 == 2 and N2 == 2 * N3 and sum(ROWS) == M and U1 == U2 and U2 * DH == D and U3 * DH == 2 * D


def _rng(s):
    a, b = s.split("-")
    return int(a), int(b)


def _parse_ops(s):
    out = []
    for t in s.split():
        if t[:2] == "QS":
            h, k = t[2:].split(":")
            out.append(("QS", _rng(h) + _rng(k)))
        else:
            out.append((t[:2], int(t[2:])))
    return out


def _parse_dmas(s):
    out = []
    for t in s.split():
        body = t[1:].split(":")
        out.append((t[0], _rng(body[0]), _rng(body[1]) if len(body) > 1 else (0, KT)))
    return out


def _chain(n, covers):
    halves = [f"{cv[0]}{ab}{cv[2:]}" for cv in covers[:n + 1] for ab in "AB"]
    o = [halves[0]]
    for j in range(n):
        o += [halves[2 * j + 1], f"TS{j}", halves[2 * j + 2], f"MM{j}"]
    return _parse_ops(" ".join(o + [halves[-1]] + covers[n + 1:]))


_START = [(_parse_dmas(s.split("|")[0]), _parse_ops(s.split("|")[1])) for s in START]
_ORD1 = _parse_ops("ZZ0 " + " ".join(f"QP{j}" for j in range(U1)))
_ORD2 = _chain(U2, [f"QP{j}" for j in range(P2)] + [f"OP{j}" for j in range(U2 - 1)] + [f"OW{U2 - 1}"])
_ORD3 = _chain(U3, [f"QP{j}" for j in range(L3)] + [f"OP{j}" for j in range(U3 - NFF)] + [f"FF{U3 - NFF}"])
_ROFF = [sum(ROWS[:t]) for t in range(len(ROWS))]

SEM1 = sum(len(d) for d, _ in _START)
SEMX = SEM1 + N1
SEM2 = SEMX + 1
SEM3 = SEM2 + 2 * N2
SEMA = SEM3 + 2 * N3
SEMO = SEMA + 1
NSEM = SEMO + len(ROWS)


def _kernel(xa, ka, va, wqa, woa, xb, kb, vb, wqb, wob, out_hbm,
            x_buf, wq_s, wq_1, w_2, w_3, k_0, kv, acc, out_a, out_b,
            q_a, q_b, q_l, q_f, p_buf, o_buf, qa_buf, sems):
    c = (DH ** -0.5) * LOG2E
    copy = pltpu.make_async_copy

    def kv_copies(g0, n, sem):
        cps = []
        for which, srcs, lo in ((0, (va, vb), g0), (1, (ka, kb), g0 + 1)):
            slot, g = g0, lo
            while slot < g0 + n:
                br, h = (g // H) % 2, g % H
                m = min(g0 + n - slot, H - h)
                cps.append(copy(srcs[br].at[:, pl.ds(h, m)], kv.at[which, :, pl.ds(slot, m)], sem))
                slot, g = slot + m, g + m
        return cps

    def outa_dma():
        return copy(out_a, out_hbm.at[:, pl.ds(0, D)], sems.at[SEMA])

    def outb_dma(t):
        rs = pl.ds(_ROFF[t], ROWS[t])
        return copy(out_b.at[rs, :], out_hbm.at[rs, pl.ds(D, D)], sems.at[SEMO + t])

    def start_copies():
        cps, si = [], 0
        for dl, _ in _START:
            seg = []
            for kind, (lo, hi), (k0, k1) in dl:
                cs = pl.ds(lo * 128, (hi - lo) * 128)
                if kind == "x":
                    seg.append(copy(xa.at[:, cs], x_buf.at[0, :, cs], sems.at[si]))
                elif kind == "q":
                    rs = pl.ds(k0 * 128, (k1 - k0) * 128)
                    seg.append(copy(wqa.at[rs, cs], wq_s.at[rs, cs], sems.at[si]))
                else:
                    seg.append(copy(ka.at[:, 0], k_0, sems.at[si]))
                si += 1
            cps.append(seg)
        return cps

    for seg in start_copies():
        for cp in seg:
            cp.start()
    for i in range(N1):
        copy(wqa.at[:, pl.ds((S + i * U1) * DH, U1 * DH)], wq_1.at[i, :, pl.ds(0, U1 * DH)], sems.at[SEM1 + i]).start()
    copy(xb, x_buf.at[1], sems.at[SEMX]).start()
    for i in range(N2):
        lo = i * P2 + (i // 2) * L3
        sem = sems.at[SEM2 + 2 * i]
        copy(wqb.at[:, pl.ds(lo * DH, P2 * DH)], w_2.at[i, :, pl.ds(D, P2 * DH)], sem).start()
        copy(woa.at[pl.ds(i * D, D), :], w_2.at[i, :, pl.ds(0, D)], sem).start()
        for cp in kv_copies(i * U2, U2, sems.at[SEM2 + 2 * i + 1]):
            cp.start()
    for i in range(N3):
        sem = sems.at[SEM3 + 2 * i]
        hw = (L3 // 2) * DH
        for r in range(2):
            copy(wqb.at[:, pl.ds(((i + 1) * U3 - L3) * DH + r * hw, hw)],
                 w_3.at[i, pl.ds(r * D, D), pl.ds(D, hw)], sem).start()
        copy(wob.at[pl.ds(i * 2 * D, 2 * D), :], w_3.at[i, :, pl.ds(0, D)], sem).start()
        for cp in kv_copies(H + i * U3, U3, sems.at[SEM3 + 2 * i + 1]):
            cp.start()

    def run(order, phase, it):
        colb = lax.broadcasted_iota(jnp.int32, (SQ, 128), 1) // SK
        colh = lax.broadcasted_iota(jnp.int32, (SQ // 2, 128), 1) // SK
        zero = jnp.zeros((SQ // 2, 128), U32)
        pbr = 0 if phase < 2 else 1
        abr = 0 if phase < 3 else 1
        n_att = {2: U2, 3: U3}.get(phase)
        st = {}

        def u32(a):
            return pltpu.bitcast(a, U32)

        def bf16(a):
            return pltpu.bitcast(a, BF16)

        def sel(i, a, b):
            return bf16(jnp.where(colh == i, u32(a), u32(b)))

        def keep(i, a):
            return bf16(jnp.where(colh != i, zero, u32(a)))

        def drop(i, a):
            return bf16(jnp.where(colh == i, zero, u32(a)))

        def blk(a, i):
            return a[i * SQ:(i + 1) * SQ, :]

        def compact(parts):
            r = parts[GB - 1]
            for i in range(GB - 2, -1, -1):
                r = jnp.where(colb == i, parts[i], r)
            return r

        def wq_tile(j, ks):
            if phase == 1:
                return wq_1[it, ks, j * DH:(j + 1) * DH]
            if phase == 2:
                return w_2[it, ks, D + j * DH:D + (j + 1) * DH]
            r, jj = divmod(j, L3 // 2)
            return w_3[it, r * D + ks.start:r * D + ks.stop, D + jj * DH:D + (jj + 1) * DH]

        def wo_rows(j, n, ns=slice(0, D)):
            return (w_2 if phase == 2 else w_3)[it, j * DH:(j + n) * DH, ns]

        def store_q(j, q):
            q = u32(q.astype(BF16))
            if phase == 0:
                if j % U2 == 0:
                    q_f[j // U2] = q
                else:
                    q_a[j] = q
            elif phase == 1:
                if j == 0:
                    q_f[S // U2 + it] = q
                else:
                    q_a[S + it * U1 + j] = q
            elif phase == 2:
                if j == 0:
                    q_f[N2 + it] = q
                q_b[it * P2 + lax.shift_right_logical(it, 1) * L3 + j] = q
            else:
                q_l[j] = q

        def q_next(j, t):
            rs = slice(t * 64, (t + 1) * 64)
            if j + 1 == n_att:
                return bf16(q_f[it + 1 if phase == 2 else N2 + 2, rs, :])
            if phase == 2:
                return bf16(q_a[it * U2 + j + 1, rs, :])
            if j + 1 >= U3 - L3:
                return bf16(q_l[j + 1 - (U3 - L3), rs, :])
            return bf16(q_b[it * U3 + j + 1, rs, :])

        def kv_tile(which, j, t):
            return kv[which, t * GB:(t + 1) * GB, abr * H + it * n_att + j].reshape(128, DH)

        def softmax(sc):
            mc = compact([jnp.max(jnp.where(colb == i, sc, -jnp.inf), axis=-1, keepdims=True)
                          for i in range(GB)])
            e = jnp.exp2((sc - mc) * c)
            lc = compact([jnp.sum(jnp.where(colb == i, e, 0.0), axis=-1, keepdims=True)
                          for i in range(GB)])
            return (e * pl.reciprocal(lc, approx=False, full_range=False)).astype(BF16)

        for op, j in order:
            if op in ("QP", "QA", "QB"):
                ks = {"QP": slice(0, D), "QA": slice(0, D // 2), "QB": slice(D // 2, D)}[op]
                q = jnp.dot(x_buf[pbr, :, ks], wq_tile(j, ks), preferred_element_type=F32)
                if op == "QA":
                    st["qa"] = q
                else:
                    store_q(j, st["qa"] + q if op == "QB" else q)
            elif op == "QS":
                ja, jb, k0, k1 = j
                q = jnp.dot(x_buf[0, :, k0 * 128:k1 * 128], wq_s[k0 * 128:k1 * 128, ja * DH:jb * DH],
                            preferred_element_type=F32)
                for jj in range(ja, jb):
                    qq = q[:, (jj - ja) * DH:(jj - ja + 1) * DH]
                    if k0 > 0:
                        qq = qa_buf[jj] + qq
                    if k1 == KT:
                        store_q(jj, qq)
                    else:
                        qa_buf[jj] = qq
            elif op == "ZZ":
                acc[it] = jnp.zeros((M, D), F32)
            elif op == "QK":
                for t in range(NG):
                    s = lax.dot_general(bf16(q_f[0, t * 64:(t + 1) * 64, :]),
                                        k_0[t * GB:(t + 1) * GB].reshape(128, DH),
                                        (((1,), (1,)), ((), ())), preferred_element_type=F32)
                    p_buf[t] = u32(softmax(compact([blk(s, i) for i in range(GB)])))
            elif op == "TS":
                for t in range(NG):
                    kt = kv_tile(1, j, t).T
                    q = q_next(j, t)
                    qc = blk(q, GB - 1)
                    for i in range(GB - 2, -1, -1):
                        qc = sel(i, blk(q, i), qc)
                    wdk = jnp.concatenate([keep(i, blk(kt, i)) for i in range(GB)], axis=0)
                    st["ts", t] = (jnp.dot(qc, wdk, preferred_element_type=F32), kt)
            elif op == "MM":
                for t in range(NG):
                    tail_s, kt = st["ts", t]
                    v = kv_tile(0, j, t)
                    q = q_next(j, t)
                    pc = bf16(p_buf[t]) if j == 0 else st["p", t]
                    wdv = jnp.concatenate([keep(i, blk(v, i)) for i in range(GB)], axis=0)
                    tail_o = jnp.dot(pc, wdv, preferred_element_type=F32)
                    mains = []
                    for i in range(GB):
                        w = jnp.concatenate(
                            [drop(i, blk(v, i)) if r == i else keep(i, blk(kt, r)) for r in range(GB)], axis=0)
                        mains.append(jnp.dot(sel(i, pc, blk(q, i)), w, preferred_element_type=F32))
                    pn = softmax(compact(mains) + tail_s)
                    if j + 1 == n_att:
                        p_buf[t] = u32(pn)
                    else:
                        st["p", t] = pn
                    o = jnp.concatenate([jnp.where(colb == i, tail_o, mains[i]) for i in range(GB)], axis=0)
                    o_buf[t * 128:(t + 1) * 128, j * DH:(j + 1) * DH] = o.astype(BF16)
            elif op in ("OP", "OW", "OA", "OB"):
                ns = {"OA": slice(0, D // 2), "OB": slice(D // 2, D)}.get(op, slice(0, D))
                r = acc[abr, :, ns] + jnp.dot(o_buf[:, j * DH:(j + 1) * DH], wo_rows(j, 1, ns),
                                              preferred_element_type=F32)
                acc[abr, :, ns] = r
                if op == "OW":
                    out_a[...] = r.astype(BF16)
            else:
                for t in range(len(ROWS)):
                    rs = slice(_ROFF[t], _ROFF[t] + ROWS[t])
                    r = acc[abr, rs, :] + jnp.dot(o_buf[rs, j * DH:U3 * DH], wo_rows(j, U3 - j),
                                                  preferred_element_type=F32)
                    acc[abr, rs, :] = r
                    out_b[rs, :] = r.astype(BF16)

                    @pl.when(it == N3 - 1)
                    def _():
                        outb_dma(t).start()

    def wait(r, sem):
        copy(r, r, sems.at[sem]).wait()

    def body1(i, carry):
        wait(wq_1.at[i, :, pl.ds(0, U1 * DH)], SEM1 + i)
        run(_ORD1, 1, i)
        return carry

    def body2(i, carry):
        wait(w_2.at[i, :, pl.ds(0, D + P2 * DH)], SEM2 + 2 * i)
        wait(kv.at[:, :, pl.ds(i * U2, U2)], SEM2 + 2 * i + 1)
        run(_ORD2, 2, i)
        return carry

    def body3(i, carry):
        wait(w_3.at[i, :, pl.ds(0, D + (L3 // 2) * DH)], SEM3 + 2 * i)
        wait(kv.at[:, :, pl.ds(H + i * U3, U3)], SEM3 + 2 * i + 1)
        run(_ORD3, 3, i)
        return carry

    def outer(ph, carry):
        @pl.when(ph == 0)
        def _():
            for seg, (_, ops) in zip(start_copies(), _START):
                for cp in seg:
                    cp.wait()
                run(ops, 0, None)
            lax.fori_loop(0, N1, body1, 0)
            wait(x_buf.at[1], SEMX)
            lax.fori_loop(0, N2, body2, 0)
            outa_dma().start()

        @pl.when(ph == 1)
        def _():
            lax.fori_loop(0, N3, body3, 0)
        return carry

    lax.fori_loop(0, 2, outer, 0)
    outa_dma().wait()
    for t in range(len(ROWS)):
        outb_dma(t).wait()


@jax.jit
def pallas_concat_heads__mha_block_cached__mha_block_cached__near_ridge_kernel(
    A_x: jax.Array,
    A_k_cache: jax.Array,
    A_v_cache: jax.Array,
    A_wq: jax.Array,
    A_wo: jax.Array,
    B_x: jax.Array,
    B_k_cache: jax.Array,
    B_v_cache: jax.Array,
    B_wq: jax.Array,
    B_wo: jax.Array,
):
    any_spec = pl.BlockSpec(memory_space=pl.ANY)
    out = pl.pallas_call(
        _kernel,
        in_specs=[any_spec] * 10,
        out_specs=any_spec,
        out_shape=jax.ShapeDtypeStruct((M, 2 * D), BF16),
        scratch_shapes=[
            pltpu.VMEM((2, M, D), BF16),
            pltpu.VMEM((D, S * DH + PAD), BF16),
            pltpu.VMEM((N1, D, U1 * DH + PAD), BF16),
            pltpu.VMEM((N2, D, W2), BF16),
            pltpu.VMEM((N3, 2 * D, W3), BF16),
            pltpu.VMEM((B, SK, DH), BF16),
            pltpu.VMEM((2, B, 2 * H, SK, DH), BF16),
            pltpu.VMEM((2, M, D), F32),
            pltpu.VMEM((M, D), BF16),
            pltpu.VMEM((M, D), BF16),
            pltpu.VMEM((H, M // 2, DH), U32),
            pltpu.VMEM((H, M // 2, DH), U32),
            pltpu.VMEM((L3, M // 2, DH), U32),
            pltpu.VMEM((2 * N2, M // 2, DH), U32),
            pltpu.VMEM((NG, SQ // 2, 128), U32),
            pltpu.VMEM((M, U3 * DH), BF16),
            pltpu.VMEM((S, M, DH), F32),
            pltpu.SemaphoreType.DMA((NSEM,)),
        ],
        compiler_params=pltpu.CompilerParams(
            vmem_limit_bytes=110 * 1024 * 1024,
            disable_bounds_checks=True,
            disable_semaphore_checks=True,
        ),
    )(A_x.reshape(M, D), A_k_cache, A_v_cache, A_wq, A_wo,
      B_x.reshape(M, D), B_k_cache, B_v_cache, B_wq, B_wo)
    return out.reshape(B, SQ, 2 * D)
```

```python
import jax
import jax.numpy as jnp
from jax import lax
import jax.experimental.pallas as pl
import jax.experimental.pallas.tpu as pltpu

B, SQ, D = 16, 32, 1024
H, SK, DH = 32, 32, 128
M = B * SQ
GB = 4
NG = B // GB
KT = D // 128
LOG2E = 1.4426950408889634
F32 = jnp.float32
BF16 = jnp.bfloat16
U32 = jnp.uint32
PAD = 128

START = [
    "x0-1 q0-8:0-1 | QS0-8:0-1",
    "q8-16:0-1 x1-2 q0-4:1-2 | QS8-16:0-1 QS0-4:1-2",
    "q4-16:1-2 x2-3 q0-8:2-3 | QS4-16:1-2 QS0-8:2-3",
    "q8-16:2-3 x3-5 q0-16:3-4 q0-12:4-5 | QS8-12:2-5 QS12-16:2-4 QS0-8:3-5",
    "q12-16:4-5 x5-8 q0-16:5-8 k0-1 | QS0-8:5-8 QS8-12:5-8 QK0 QS12-16:4-8",
]
S = 16
U2 = 8
N2 = S // U2
U3 = 16
N3 = (2 * H - S) // U3
L3 = 6
U1 = U3 - L3
N1 = 2
P2 = U1 // N2
NFF = 3
ROWS = (160, 128, 96, 64, 32, 32)
W1 = U1 * DH + (PAD if U1 % 2 == 0 else 0)
W2 = D + P2 * DH + (PAD if P2 % 2 == 0 else 0)
W3 = D + (L3 // 2) * DH + (PAD if (L3 // 2) % 2 == 0 else 0)
assert N2 == 2 and N3 == 3 and sum(ROWS) == M and U2 * DH == D and U3 * DH == 2 * D and P2 * N2 == U1


def _rng(s):
    a, b = s.split("-")
    return int(a), int(b)


def _parse_ops(s):
    out = []
    for t in s.split():
        if t[:2] == "QS":
            h, k = t[2:].split(":")
            out.append(("QS", _rng(h) + _rng(k)))
        else:
            out.append((t[:2], int(t[2:])))
    return out


def _parse_dmas(s):
    out = []
    for t in s.split():
        body = t[1:].split(":")
        out.append((t[0], _rng(body[0]), _rng(body[1]) if len(body) > 1 else (0, KT)))
    return out


def _chain(n, covers):
    halves = [f"{cv[0]}{ab}{cv[2:]}" for cv in covers[:n + 1] for ab in "AB"]
    o = [halves[0]]
    for j in range(n):
        o += [halves[2 * j + 1], f"TS{j}", halves[2 * j + 2], f"MM{j}"]
    return _parse_ops(" ".join(o + [halves[-1]] + covers[n + 1:]))


_START = [(_parse_dmas(s.split("|")[0]), _parse_ops(s.split("|")[1])) for s in START]
_ORD1 = _parse_ops("ZZ0 " + " ".join(f"QP{j}" for j in range(U1)))
_ORD2 = _chain(U2, [f"QP{j}" for j in range(P2)] + [f"OP{j}" for j in range(U2)])
_ORD3 = _chain(U3, [f"QP{j}" for j in range(L3)] + [f"OP{j}" for j in range(U3 - NFF)] + [f"FF{U3 - NFF}"])
_ROFF = [sum(ROWS[:t]) for t in range(len(ROWS))]

SEM1 = sum(len(d) for d, _ in _START)
SEMX = SEM1 + N1
SEM2 = SEMX + 1
SEM3 = SEM2 + 2 * N2
SEMO = SEM3 + 2 * N3
NSEM = SEMO + 2 * len(ROWS)


def _kernel(xa, ka, va, wqa, woa, xb, kb, vb, wqb, wob, out_hbm,
            x_buf, wq_s, wq_1, w_2, w_3, k_0, kv, acc, out_buf,
            q_s, q_n, q_l, q_f, p_buf, o_buf, qa_buf, sems):
    c = (DH ** -0.5) * LOG2E
    copy = pltpu.make_async_copy

    def kv_copies(g0, n, sem):
        cps = []
        for which, srcs, lo in ((0, (va, vb), g0), (1, (ka, kb), g0 + 1)):
            slot, g = g0, lo
            while slot < g0 + n:
                br, h = (g // H) % 2, g % H
                m = min(g0 + n - slot, H - h)
                cps.append(copy(srcs[br].at[:, pl.ds(h, m)], kv.at[which, :, pl.ds(slot, m)], sem))
                slot, g = slot + m, g + m
        return cps

    def out_dma(br, t):
        rs = pl.ds(_ROFF[t], ROWS[t])
        return copy(out_buf.at[br, rs, :], out_hbm.at[rs, pl.ds(pl.multiple_of(br * D, D), D)],
                    sems.at[SEMO + br * len(ROWS) + t])

    def src(g):
        return ((wqa, woa), (wqb, wob))[g // H] + ((g % H) * DH,)

    def start_copies():
        cps, si = [], 0
        for dl, _ in _START:
            seg = []
            for kind, (lo, hi), (k0, k1) in dl:
                cs = pl.ds(lo * 128, (hi - lo) * 128)
                if kind == "x":
                    seg.append(copy(xa.at[:, cs], x_buf.at[0, :, cs], sems.at[si]))
                elif kind == "q":
                    rs = pl.ds(k0 * 128, (k1 - k0) * 128)
                    seg.append(copy(wqa.at[rs, cs], wq_s.at[rs, cs], sems.at[si]))
                else:
                    seg.append(copy(ka.at[:, 0], k_0, sems.at[si]))
                si += 1
            cps.append(seg)
        return cps

    for seg in start_copies():
        for cp in seg:
            cp.start()
    for i in range(N1):
        if i == 1:
            copy(xb, x_buf.at[1], sems.at[SEMX]).start()
        wq, _, lo = src(S + i * U3)
        copy(wq.at[:, pl.ds(lo, U1 * DH)], wq_1.at[i, :, pl.ds(0, U1 * DH)], sems.at[SEM1 + i]).start()
    for i in range(N2):
        sem = sems.at[SEM2 + 2 * i]
        wq, _, lo = src(S + N1 * U3 + i * P2)
        copy(wq.at[:, pl.ds(lo, P2 * DH)], w_2.at[i, :, pl.ds(D, P2 * DH)], sem).start()
        copy(woa.at[pl.ds(i * D, D), :], w_2.at[i, :, pl.ds(0, D)], sem).start()
        for cp in kv_copies(i * U2, U2, sems.at[SEM2 + 2 * i + 1]):
            cp.start()
    for i in range(N3):
        sem = sems.at[SEM3 + 2 * i]
        wq, wo, lo = src(S + i * U3)
        hw = (L3 // 2) * DH
        for r in range(2):
            copy(wq.at[:, pl.ds(lo + U1 * DH + r * hw, hw)], w_3.at[i, pl.ds(r * D, D), pl.ds(D, hw)], sem).start()
        copy(wo.at[pl.ds(lo, 2 * D), :], w_3.at[i, :, pl.ds(0, D)], sem).start()
        for cp in kv_copies(S + i * U3, U3, sems.at[SEM3 + 2 * i + 1]):
            cp.start()

    def run(order, phase, it):
        colb = lax.broadcasted_iota(jnp.int32, (SQ, 128), 1) // SK
        colh = lax.broadcasted_iota(jnp.int32, (SQ // 2, 128), 1) // SK
        zero = jnp.zeros((SQ // 2, 128), U32)
        br3 = jnp.minimum(it, 1) if phase == 3 else None
        pbr = {0: 0, 1: it, 2: 1, 3: br3}[phase]
        abr = br3 if phase == 3 else 0
        n_att = {2: U2, 3: U3}.get(phase)
        st = {}

        def u32(a):
            return pltpu.bitcast(a, U32)

        def bf16(a):
            return pltpu.bitcast(a, BF16)

        def sel(i, a, b):
            return bf16(jnp.where(colh == i, u32(a), u32(b)))

        def keep(i, a):
            return bf16(jnp.where(colh != i, zero, u32(a)))

        def drop(i, a):
            return bf16(jnp.where(colh == i, zero, u32(a)))

        def blk(a, i):
            return a[i * SQ:(i + 1) * SQ, :]

        def compact(parts):
            r = parts[GB - 1]
            for i in range(GB - 2, -1, -1):
                r = jnp.where(colb == i, parts[i], r)
            return r

        def wq_tile(j, ks):
            if phase == 1:
                return wq_1[it, ks, j * DH:(j + 1) * DH]
            if phase == 2:
                return w_2[it, ks, D + j * DH:D + (j + 1) * DH]
            r, jj = divmod(j, L3 // 2)
            return w_3[it, r * D + ks.start:r * D + ks.stop, D + jj * DH:D + (jj + 1) * DH]

        def wo_rows(j, n, ns=slice(0, D)):
            return (w_2 if phase == 2 else w_3)[it, j * DH:(j + n) * DH, ns]

        def store_q(j, q):
            q = u32(q.astype(BF16))
            if phase == 0:
                if j % U2 == 0:
                    q_f[j // U2] = q
                else:
                    q_s[j] = q
            elif phase == 1:
                if j == 0:
                    q_f[N2 + it] = q
                q_n[it * U1 + j] = q
            elif phase == 2:
                q_n[N1 * U1 + it * P2 + j] = q
            else:
                q_l[j] = q

        def q_next(j, t):
            rs = slice(t * 64, (t + 1) * 64)
            if phase == 2:
                return bf16(q_f[it + 1, rs, :] if j + 1 == U2 else q_s[it * U2 + j + 1, rs, :])
            if j + 1 == U3:
                return bf16(q_n[(br3 + 1) * U1, rs, :])
            if j + 1 >= U1:
                return bf16(q_l[j + 1 - U1, rs, :])
            return bf16(q_n[it * U1 + j + 1, rs, :])

        def kv_tile(which, j, t):
            g0 = it * U2 if phase == 2 else S + it * U3
            return kv[which, t * GB:(t + 1) * GB, g0 + j].reshape(128, DH)

        def softmax(sc):
            mc = compact([jnp.max(jnp.where(colb == i, sc, -jnp.inf), axis=-1, keepdims=True)
                          for i in range(GB)])
            e = jnp.exp2((sc - mc) * c)
            lc = compact([jnp.sum(jnp.where(colb == i, e, 0.0), axis=-1, keepdims=True)
                          for i in range(GB)])
            return (e * pl.reciprocal(lc, approx=False, full_range=False)).astype(BF16)

        for op, j in order:
            if op in ("QP", "QA", "QB"):
                ks = {"QP": slice(0, D), "QA": slice(0, D // 2), "QB": slice(D // 2, D)}[op]
                q = jnp.dot(x_buf[pbr, :, ks], wq_tile(j, ks), preferred_element_type=F32)
                if op == "QA":
                    st["qa"] = q
                else:
                    store_q(j, st["qa"] + q if op == "QB" else q)
            elif op == "QS":
                ja, jb, k0, k1 = j
                q = jnp.dot(x_buf[0, :, k0 * 128:k1 * 128], wq_s[k0 * 128:k1 * 128, ja * DH:jb * DH],
                            preferred_element_type=F32)
                for jj in range(ja, jb):
                    qq = q[:, (jj - ja) * DH:(jj - ja + 1) * DH]
                    if k0 > 0:
                        qq = qa_buf[jj] + qq
                    if k1 == KT:
                        store_q(jj, qq)
                    else:
                        qa_buf[jj] = qq
            elif op == "ZZ":
                acc[it] = jnp.zeros((M, D), F32)
            elif op == "QK":
                for t in range(NG):
                    s = lax.dot_general(bf16(q_f[0, t * 64:(t + 1) * 64, :]),
                                        k_0[t * GB:(t + 1) * GB].reshape(128, DH),
                                        (((1,), (1,)), ((), ())), preferred_element_type=F32)
                    p_buf[t] = u32(softmax(compact([blk(s, i) for i in range(GB)])))
            elif op == "TS":
                for t in range(NG):
                    kt = kv_tile(1, j, t).T
                    q = q_next(j, t)
                    qc = blk(q, GB - 1)
                    for i in range(GB - 2, -1, -1):
                        qc = sel(i, blk(q, i), qc)
                    wdk = jnp.concatenate([keep(i, blk(kt, i)) for i in range(GB)], axis=0)
                    st["ts", t] = (jnp.dot(qc, wdk, preferred_element_type=F32), kt)
            elif op == "MM":
                for t in range(NG):
                    tail_s, kt = st["ts", t]
                    v = kv_tile(0, j, t)
                    q = q_next(j, t)
                    pc = bf16(p_buf[t]) if j == 0 else st["p", t]
                    wdv = jnp.concatenate([keep(i, blk(v, i)) for i in range(GB)], axis=0)
                    tail_o = jnp.dot(pc, wdv, preferred_element_type=F32)
                    mains = []
                    for i in range(GB):
                        w = jnp.concatenate(
                            [drop(i, blk(v, i)) if r == i else keep(i, blk(kt, r)) for r in range(GB)], axis=0)
                        mains.append(jnp.dot(sel(i, pc, blk(q, i)), w, preferred_element_type=F32))
                    pn = softmax(compact(mains) + tail_s)
                    if j + 1 == n_att:
                        p_buf[t] = u32(pn)
                    else:
                        st["p", t] = pn
                    o = jnp.concatenate([jnp.where(colb == i, tail_o, mains[i]) for i in range(GB)], axis=0)
                    o_buf[t * 128:(t + 1) * 128, j * DH:(j + 1) * DH] = o.astype(BF16)
            elif op in ("OP", "OA", "OB"):
                ns = {"OA": slice(0, D // 2), "OB": slice(D // 2, D)}.get(op, slice(0, D))
                r = acc[abr, :, ns] + jnp.dot(o_buf[:, j * DH:(j + 1) * DH], wo_rows(j, 1, ns),
                                              preferred_element_type=F32)
                acc[abr, :, ns] = r
            else:
                for t in range(len(ROWS)):
                    rs = slice(_ROFF[t], _ROFF[t] + ROWS[t])
                    r = acc[abr, rs, :] + jnp.dot(o_buf[rs, j * DH:U3 * DH], wo_rows(j, U3 - j),
                                                  preferred_element_type=F32)
                    acc[abr, rs, :] = r
                    out_buf[abr, rs, :] = r.astype(BF16)

                    @pl.when(it != 1)
                    def _():
                        out_dma(abr, t).start()

    def wait(r, sem):
        copy(r, r, sems.at[sem]).wait()

    def body1(i, carry):
        @pl.when(i == 1)
        def _():
            wait(x_buf.at[1], SEMX)

        wait(wq_1.at[i, :, pl.ds(0, U1 * DH)], SEM1 + i)
        run(_ORD1, 1, i)
        return carry

    def body2(i, carry):
        wait(w_2.at[i, :, pl.ds(0, D + P2 * DH)], SEM2 + 2 * i)
        wait(kv.at[:, :, pl.ds(i * U2, U2)], SEM2 + 2 * i + 1)
        run(_ORD2, 2, i)
        return carry

    def body3(i, carry):
        wait(w_3.at[i, :, pl.ds(0, D + (L3 // 2) * DH)], SEM3 + 2 * i)
        wait(kv.at[:, :, pl.ds(S + i * U3, U3)], SEM3 + 2 * i + 1)
        run(_ORD3, 3, i)
        return carry

    def outer(ph, carry):
        @pl.when(ph == 0)
        def _():
            for seg, (_, ops) in zip(start_copies(), _START):
                for cp in seg:
                    cp.wait()
                run(ops, 0, None)
            lax.fori_loop(0, N1, body1, 0)
            lax.fori_loop(0, N2, body2, 0)

        @pl.when(ph == 1)
        def _():
            lax.fori_loop(0, N3, body3, 0)
        return carry

    lax.fori_loop(0, 2, outer, 0)
    for br in range(2):
        for t in range(len(ROWS)):
            out_dma(br, t).wait()


@jax.jit
def pallas_concat_heads__mha_block_cached__mha_block_cached__near_ridge_kernel(
    A_x: jax.Array,
    A_k_cache: jax.Array,
    A_v_cache: jax.Array,
    A_wq: jax.Array,
    A_wo: jax.Array,
    B_x: jax.Array,
    B_k_cache: jax.Array,
    B_v_cache: jax.Array,
    B_wq: jax.Array,
    B_wo: jax.Array,
):
    any_spec = pl.BlockSpec(memory_space=pl.ANY)
    out = pl.pallas_call(
        _kernel,
        in_specs=[any_spec] * 10,
        out_specs=any_spec,
        out_shape=jax.ShapeDtypeStruct((M, 2 * D), BF16),
        scratch_shapes=[
            pltpu.VMEM((2, M, D), BF16),
            pltpu.VMEM((D, S * DH + PAD), BF16),
            pltpu.VMEM((N1, D, W1), BF16),
            pltpu.VMEM((N2, D, W2), BF16),
            pltpu.VMEM((N3, 2 * D, W3), BF16),
            pltpu.VMEM((B, SK, DH), BF16),
            pltpu.VMEM((2, B, 2 * H, SK, DH), BF16),
            pltpu.VMEM((2, M, D), F32),
            pltpu.VMEM((2, M, D), BF16),
            pltpu.VMEM((S, M // 2, DH), U32),
            pltpu.VMEM((N3 * U1, M // 2, DH), U32),
            pltpu.VMEM((L3, M // 2, DH), U32),
            pltpu.VMEM((N2 + N1, M // 2, DH), U32),
            pltpu.VMEM((NG, SQ // 2, 128), U32),
            pltpu.VMEM((M, U3 * DH), BF16),
            pltpu.VMEM((S, M, DH), F32),
            pltpu.SemaphoreType.DMA((NSEM,)),
        ],
        compiler_params=pltpu.CompilerParams(
            vmem_limit_bytes=110 * 1024 * 1024,
            disable_bounds_checks=True,
            disable_semaphore_checks=True,
        ),
    )(A_x.reshape(M, D), A_k_cache, A_v_cache, A_wq, A_wo,
      B_x.reshape(M, D), B_k_cache, B_v_cache, B_wq, B_wo)
    return out.reshape(B, SQ, 2 * D)
```

```python
import jax
import jax.numpy as jnp
from jax import lax
import jax.experimental.pallas as pl
import jax.experimental.pallas.tpu as pltpu

B, SQ, D = 16, 32, 1024
H, SK, DH = 32, 32, 128
M = B * SQ
GB = 4
NG = B // GB
KT = D // 128
LOG2E = 1.4426950408889634
F32 = jnp.float32
BF16 = jnp.bfloat16
U32 = jnp.uint32
PAD = 128

START = [
    "x0-1 q0-4:0-1 | QS0-4:0-1",
    "q4-12:0-1 | QS4-12:0-1",
    "q12-16:0-1 x1-2 q0-8:1-2 | QS12-16:0-1 QS0-8:1-2",
    "q8-16:1-2 x2-3 q0-12:2-3 | QS8-12:1-3 QS12-16:1-2 QS0-8:2-3",
    "q12-16:2-3 x3-5 q0-16:3-5 | QS12-16:2-5 QS0-12:3-5",
    "x5-8 q0-16:5-8 k0-1 | QS0-12:5-8 QK0 QS12-16:5-8",
]
S = 16
U2 = 8
N2 = S // U2
U3 = 16
N3 = (2 * H - S) // U3
L3 = 6
U1 = U3 - L3
N1 = 2
P2 = U1 // N2
NFF = 3
ROWS = (160, 128, 96, 64, 32, 32)
W1 = U1 * DH + (PAD if U1 % 2 == 0 else 0)
W2 = D + P2 * DH + (PAD if P2 % 2 == 0 else 0)
W3 = D + (L3 // 2) * DH + (PAD if (L3 // 2) % 2 == 0 else 0)
assert N2 == 2 and N3 == 3 and sum(ROWS) == M and U2 * DH == D and U3 * DH == 2 * D and P2 * N2 == U1


def _rng(s):
    a, b = s.split("-")
    return int(a), int(b)


def _parse_ops(s):
    out = []
    for t in s.split():
        if t[:2] == "QS":
            h, k = t[2:].split(":")
            out.append(("QS", _rng(h) + _rng(k)))
        else:
            out.append((t[:2], int(t[2:])))
    return out


def _parse_dmas(s):
    out = []
    for t in s.split():
        body = t[1:].split(":")
        out.append((t[0], _rng(body[0]), _rng(body[1]) if len(body) > 1 else (0, KT)))
    return out


def _chain(n, covers):
    halves = [f"{cv[0]}{ab}{cv[2:]}" for cv in covers[:n + 1] for ab in "AB"]
    o = [halves[0]]
    for j in range(n):
        o += [halves[2 * j + 1], f"TS{j}", halves[2 * j + 2], f"MM{j}"]
    return _parse_ops(" ".join(o + [halves[-1]] + covers[n + 1:]))


_START = [(_parse_dmas(s.split("|")[0]), _parse_ops(s.split("|")[1])) for s in START]
_ORD1 = _parse_ops("ZZ0 " + " ".join(f"QP{j}" for j in range(U1)))
_ORD2 = _chain(U2, [f"QP{j}" for j in range(P2)] + [f"OP{j}" for j in range(U2)])
_ORD3 = _chain(U3, [f"QP{j}" for j in range(L3)] + [f"OP{j}" for j in range(U3 - NFF)] + [f"FF{U3 - NFF}"])
_ROFF = [sum(ROWS[:t]) for t in range(len(ROWS))]

SEM1 = sum(len(d) for d, _ in _START)
SEMX = SEM1 + N1
SEM2 = SEMX + 1
SEM3 = SEM2 + 2 * N2
SEMO = SEM3 + 2 * N3
NSEM = SEMO + 2 * len(ROWS)


def _kernel(xa, ka, va, wqa, woa, xb, kb, vb, wqb, wob, out_hbm,
            x_buf, wq_s, wq_1, w_2, w_3, k_0, kv, acc, out_buf,
            q_s, q_n, q_l, q_f, p_buf, o_buf, qa_buf, sems):
    c = (DH ** -0.5) * LOG2E
    copy = pltpu.make_async_copy

    def kv_copies(g0, n, sem):
        cps = []
        for which, srcs, lo in ((0, (va, vb), g0), (1, (ka, kb), g0 + 1)):
            slot, g = g0, lo
            while slot < g0 + n:
                br, h = (g // H) % 2, g % H
                m = min(g0 + n - slot, H - h)
                cps.append(copy(srcs[br].at[:, pl.ds(h, m)], kv.at[which, :, pl.ds(slot, m)], sem))
                slot, g = slot + m, g + m
        return cps

    def out_dma(br, t):
        rs = pl.ds(_ROFF[t], ROWS[t])
        return copy(out_buf.at[br, rs, :], out_hbm.at[rs, pl.ds(pl.multiple_of(br * D, D), D)],
                    sems.at[SEMO + br * len(ROWS) + t])

    def src(g):
        return ((wqa, woa), (wqb, wob))[g // H] + ((g % H) * DH,)

    def start_copies():
        cps, si = [], 0
        for dl, _ in _START:
            seg = []
            for kind, (lo, hi), (k0, k1) in dl:
                cs = pl.ds(lo * 128, (hi - lo) * 128)
                if kind == "x":
                    seg.append(copy(xa.at[:, cs], x_buf.at[0, :, cs], sems.at[si]))
                elif kind == "q":
                    rs = pl.ds(k0 * 128, (k1 - k0) * 128)
                    seg.append(copy(wqa.at[rs, cs], wq_s.at[rs, cs], sems.at[si]))
                else:
                    seg.append(copy(ka.at[:, 0], k_0, sems.at[si]))
                si += 1
            cps.append(seg)
        return cps

    for seg in start_copies():
        for cp in seg:
            cp.start()
    for i in range(N1):
        if i == 1:
            copy(xb, x_buf.at[1], sems.at[SEMX]).start()
        wq, _, lo = src(S + i * U3)
        copy(wq.at[:, pl.ds(lo, U1 * DH)], wq_1.at[i, :, pl.ds(0, U1 * DH)], sems.at[SEM1 + i]).start()
    for i in range(N2):
        sem = sems.at[SEM2 + 2 * i]
        wq, _, lo = src(S + N1 * U3 + i * P2)
        copy(wq.at[:, pl.ds(lo, P2 * DH)], w_2.at[i, :, pl.ds(D, P2 * DH)], sem).start()
        copy(woa.at[pl.ds(i * D, D), :], w_2.at[i, :, pl.ds(0, D)], sem).start()
        for cp in kv_copies(i * U2, U2, sems.at[SEM2 + 2 * i + 1]):
            cp.start()
    for i in range(N3):
        sem = sems.at[SEM3 + 2 * i]
        wq, wo, lo = src(S + i * U3)
        hw = (L3 // 2) * DH
        for r in range(2):
            copy(wq.at[:, pl.ds(lo + U1 * DH + r * hw, hw)], w_3.at[i, pl.ds(r * D, D), pl.ds(D, hw)], sem).start()
        copy(wo.at[pl.ds(lo, 2 * D), :], w_3.at[i, :, pl.ds(0, D)], sem).start()
        for cp in kv_copies(S + i * U3, U3, sems.at[SEM3 + 2 * i + 1]):
            cp.start()

    def run(order, phase, it):
        colb = lax.broadcasted_iota(jnp.int32, (SQ, 128), 1) // SK
        colh = lax.broadcasted_iota(jnp.int32, (SQ // 2, 128), 1) // SK
        zero = jnp.zeros((SQ // 2, 128), U32)
        br3 = jnp.minimum(it, 1) if phase == 3 else None
        pbr = {0: 0, 1: it, 2: 1, 3: br3}[phase]
        abr = br3 if phase == 3 else 0
        n_att = {2: U2, 3: U3}.get(phase)
        st = {}

        def u32(a):
            return pltpu.bitcast(a, U32)

        def bf16(a):
            return pltpu.bitcast(a, BF16)

        def sel(i, a, b):
            return bf16(jnp.where(colh == i, u32(a), u32(b)))

        def keep(i, a):
            return bf16(jnp.where(colh != i, zero, u32(a)))

        def drop(i, a):
            return bf16(jnp.where(colh == i, zero, u32(a)))

        def blk(a, i):
            return a[i * SQ:(i + 1) * SQ, :]

        def compact(parts):
            r = parts[GB - 1]
            for i in range(GB - 2, -1, -1):
                r = jnp.where(colb == i, parts[i], r)
            return r

        def wq_tile(j, ks):
            if phase == 1:
                return wq_1[it, ks, j * DH:(j + 1) * DH]
            if phase == 2:
                return w_2[it, ks, D + j * DH:D + (j + 1) * DH]
            r, jj = divmod(j, L3 // 2)
            return w_3[it, r * D + ks.start:r * D + ks.stop, D + jj * DH:D + (jj + 1) * DH]

        def wo_rows(j, n, ns=slice(0, D)):
            return (w_2 if phase == 2 else w_3)[it, j * DH:(j + n) * DH, ns]

        def store_q(j, q):
            q = u32(q.astype(BF16))
            if phase == 0:
                if j % U2 == 0:
                    q_f[j // U2] = q
                else:
                    q_s[j] = q
            elif phase == 1:
                if j == 0:
                    q_f[N2 + it] = q
                q_n[it * U1 + j] = q
            elif phase == 2:
                q_n[N1 * U1 + it * P2 + j] = q
            else:
                q_l[j] = q

        def q_next(j, t):
            rs = slice(t * 64, (t + 1) * 64)
            if phase == 2:
                return bf16(q_f[it + 1, rs, :] if j + 1 == U2 else q_s[it * U2 + j + 1, rs, :])
            if j + 1 == U3:
                return bf16(q_n[(br3 + 1) * U1, rs, :])
            if j + 1 >= U1:
                return bf16(q_l[j + 1 - U1, rs, :])
            return bf16(q_n[it * U1 + j + 1, rs, :])

        def kv_tile(which, j, t):
            g0 = it * U2 if phase == 2 else S + it * U3
            return kv[which, t * GB:(t + 1) * GB, g0 + j].reshape(128, DH)

        def softmax(sc):
            mc = compact([jnp.max(jnp.where(colb == i, sc, -jnp.inf), axis=-1, keepdims=True)
                          for i in range(GB)])
            e = jnp.exp2((sc - mc) * c)
            lc = compact([jnp.sum(jnp.where(colb == i, e, 0.0), axis=-1, keepdims=True)
                          for i in range(GB)])
            return (e * pl.reciprocal(lc, approx=False, full_range=False)).astype(BF16)

        for op, j in order:
            if op in ("QP", "QA", "QB"):
                ks = {"QP": slice(0, D), "QA": slice(0, D // 2), "QB": slice(D // 2, D)}[op]
                q = jnp.dot(x_buf[pbr, :, ks], wq_tile(j, ks), preferred_element_type=F32)
                if op == "QA":
                    st["qa"] = q
                else:
                    store_q(j, st["qa"] + q if op == "QB" else q)
            elif op == "QS":
                ja, jb, k0, k1 = j
                q = jnp.dot(x_buf[0, :, k0 * 128:k1 * 128], wq_s[k0 * 128:k1 * 128, ja * DH:jb * DH],
                            preferred_element_type=F32)
                for jj in range(ja, jb):
                    qq = q[:, (jj - ja) * DH:(jj - ja + 1) * DH]
                    if k0 > 0:
                        qq = qa_buf[jj] + qq
                    if k1 == KT:
                        store_q(jj, qq)
                    else:
                        qa_buf[jj] = qq
            elif op == "ZZ":
                acc[it] = jnp.zeros((M, D), F32)
            elif op == "QK":
                for t in range(NG):
                    s = lax.dot_general(bf16(q_f[0, t * 64:(t + 1) * 64, :]),
                                        k_0[t * GB:(t + 1) * GB].reshape(128, DH),
                                        (((1,), (1,)), ((), ())), preferred_element_type=F32)
                    p_buf[t] = u32(softmax(compact([blk(s, i) for i in range(GB)])))
            elif op == "TS":
                for t in range(NG):
                    kt = kv_tile(1, j, t).T
                    q = q_next(j, t)
                    qc = blk(q, GB - 1)
                    for i in range(GB - 2, -1, -1):
                        qc = sel(i, blk(q, i), qc)
                    wdk = jnp.concatenate([keep(i, blk(kt, i)) for i in range(GB)], axis=0)
                    st["ts", t] = (jnp.dot(qc, wdk, preferred_element_type=F32), kt)
            elif op == "MM":
                for t in range(NG):
                    tail_s, kt = st["ts", t]
                    v = kv_tile(0, j, t)
                    q = q_next(j, t)
                    pc = bf16(p_buf[t]) if j == 0 else st["p", t]
                    wdv = jnp.concatenate([keep(i, blk(v, i)) for i in range(GB)], axis=0)
                    tail_o = jnp.dot(pc, wdv, preferred_element_type=F32)
                    mains = []
                    for i in range(GB):
                        w = jnp.concatenate(
                            [drop(i, blk(v, i)) if r == i else keep(i, blk(kt, r)) for r in range(GB)], axis=0)
                        mains.append(jnp.dot(sel(i, pc, blk(q, i)), w, preferred_element_type=F32))
                    pn = softmax(compact(mains) + tail_s)
                    if j + 1 == n_att:
                        p_buf[t] = u32(pn)
                    else:
                        st["p", t] = pn
                    o = jnp.concatenate([jnp.where(colb == i, tail_o, mains[i]) for i in range(GB)], axis=0)
                    o_buf[t * 128:(t + 1) * 128, j * DH:(j + 1) * DH] = o.astype(BF16)
            elif op in ("OP", "OA", "OB"):
                ns = {"OA": slice(0, D // 2), "OB": slice(D // 2, D)}.get(op, slice(0, D))
                r = acc[abr, :, ns] + jnp.dot(o_buf[:, j * DH:(j + 1) * DH], wo_rows(j, 1, ns),
                                              preferred_element_type=F32)
                acc[abr, :, ns] = r
            else:
                for t in range(len(ROWS)):
                    rs = slice(_ROFF[t], _ROFF[t] + ROWS[t])
                    r = acc[abr, rs, :] + jnp.dot(o_buf[rs, j * DH:U3 * DH], wo_rows(j, U3 - j),
                                                  preferred_element_type=F32)
                    acc[abr, rs, :] = r
                    out_buf[abr, rs, :] = r.astype(BF16)

                    @pl.when(it != 1)
                    def _():
                        out_dma(abr, t).start()

    def wait(r, sem):
        copy(r, r, sems.at[sem]).wait()

    def body1(i, carry):
        @pl.when(i == 1)
        def _():
            wait(x_buf.at[1], SEMX)

        wait(wq_1.at[i, :, pl.ds(0, U1 * DH)], SEM1 + i)
        run(_ORD1, 1, i)
        return carry

    def body2(i, carry):
        wait(w_2.at[i, :, pl.ds(0, D + P2 * DH)], SEM2 + 2 * i)
        wait(kv.at[:, :, pl.ds(i * U2, U2)], SEM2 + 2 * i + 1)
        run(_ORD2, 2, i)
        return carry

    def body3(i, carry):
        wait(w_3.at[i, :, pl.ds(0, D + (L3 // 2) * DH)], SEM3 + 2 * i)
        wait(kv.at[:, :, pl.ds(S + i * U3, U3)], SEM3 + 2 * i + 1)
        run(_ORD3, 3, i)
        return carry

    def outer(ph, carry):
        @pl.when(ph == 0)
        def _():
            for seg, (_, ops) in zip(start_copies(), _START):
                for cp in seg:
                    cp.wait()
                run(ops, 0, None)
            lax.fori_loop(0, N1, body1, 0)
            lax.fori_loop(0, N2, body2, 0)

        @pl.when(ph == 1)
        def _():
            lax.fori_loop(0, N3, body3, 0)
        return carry

    lax.fori_loop(0, 2, outer, 0)
    for br in range(2):
        for t in range(len(ROWS)):
            out_dma(br, t).wait()


@jax.jit
def pallas_concat_heads__mha_block_cached__mha_block_cached__near_ridge_kernel(
    A_x: jax.Array,
    A_k_cache: jax.Array,
    A_v_cache: jax.Array,
    A_wq: jax.Array,
    A_wo: jax.Array,
    B_x: jax.Array,
    B_k_cache: jax.Array,
    B_v_cache: jax.Array,
    B_wq: jax.Array,
    B_wo: jax.Array,
):
    any_spec = pl.BlockSpec(memory_space=pl.ANY)
    out = pl.pallas_call(
        _kernel,
        in_specs=[any_spec] * 10,
        out_specs=any_spec,
        out_shape=jax.ShapeDtypeStruct((M, 2 * D), BF16),
        scratch_shapes=[
            pltpu.VMEM((2, M, D), BF16),
            pltpu.VMEM((D, S * DH + PAD), BF16),
            pltpu.VMEM((N1, D, W1), BF16),
            pltpu.VMEM((N2, D, W2), BF16),
            pltpu.VMEM((N3, 2 * D, W3), BF16),
            pltpu.VMEM((B, SK, DH), BF16),
            pltpu.VMEM((2, B, 2 * H, SK, DH), BF16),
            pltpu.VMEM((2, M, D), F32),
            pltpu.VMEM((2, M, D), BF16),
            pltpu.VMEM((S, M // 2, DH), U32),
            pltpu.VMEM((N3 * U1, M // 2, DH), U32),
            pltpu.VMEM((L3, M // 2, DH), U32),
            pltpu.VMEM((N2 + N1, M // 2, DH), U32),
            pltpu.VMEM((NG, SQ // 2, 128), U32),
            pltpu.VMEM((M, U3 * DH), BF16),
            pltpu.VMEM((S, M, DH), F32),
            pltpu.SemaphoreType.DMA((NSEM,)),
        ],
        compiler_params=pltpu.CompilerParams(
            vmem_limit_bytes=110 * 1024 * 1024,
            disable_bounds_checks=True,
            disable_semaphore_checks=True,
        ),
    )(A_x.reshape(M, D), A_k_cache, A_v_cache, A_wq, A_wo,
      B_x.reshape(M, D), B_k_cache, B_v_cache, B_wq, B_wo)
    return out.reshape(B, SQ, 2 * D)
```

```python
import jax
import jax.numpy as jnp
from jax import lax
import jax.experimental.pallas as pl
import jax.experimental.pallas.tpu as pltpu

B, SQ, D = 16, 32, 1024
H, SK, DH = 32, 32, 128
M = B * SQ
GB = 4
NG = B // GB
KT = D // 128
LOG2E = 1.4426950408889634
F32 = jnp.float32
BF16 = jnp.bfloat16
U32 = jnp.uint32
PAD = 128

START = [
    "x0-1 q0-4:0-1 | QS0-4:0-1",
    "q4-12:0-1 | QS4-12:0-1",
    "q12-16:0-1 x1-2 q0-8:1-2 | QS12-16:0-1 QS0-8:1-2",
    "q8-16:1-2 x2-3 q0-12:2-3 | QS8-12:1-3 QS12-16:1-2 QS0-8:2-3",
    "q12-16:2-3 x3-5 q0-16:3-5 | QS12-16:2-5 QS0-12:3-5",
    "x5-8 q0-16:5-8 k0-1 | QS0-12:5-8 QK0 QS12-16:5-8",
]
S = 16
U2 = 8
N2 = S // U2
U3 = 16
N3 = (2 * H - S) // U3
L3 = 6
U1 = U3 - L3
N1 = 2
P2 = U1 // N2
NFF = 3
ROWS = (160, 128, 96, 64, 32, 32)
W1 = U1 * DH + (PAD if U1 % 2 == 0 else 0)
W2 = D + P2 * DH + (PAD if P2 % 2 == 0 else 0)
W3 = D + (L3 // 2) * DH + (PAD if (L3 // 2) % 2 == 0 else 0)
assert N2 == 2 and N3 == 3 and sum(ROWS) == M and U2 * DH == D and U3 * DH == 2 * D and P2 * N2 == U1


def _rng(s):
    a, b = s.split("-")
    return int(a), int(b)


def _parse_ops(s):
    out = []
    for t in s.split():
        if t[:2] == "QS":
            h, k = t[2:].split(":")
            out.append(("QS", _rng(h) + _rng(k)))
        else:
            out.append((t[:2], int(t[2:])))
    return out


def _parse_dmas(s):
    out = []
    for t in s.split():
        body = t[1:].split(":")
        out.append((t[0], _rng(body[0]), _rng(body[1]) if len(body) > 1 else (0, KT)))
    return out


def _chain(n, covers):
    o = []
    for j in range(n):
        o += [covers[j], f"TS{j}", f"MM{j}"]
    return _parse_ops(" ".join(o + covers[n:]))


_START = [(_parse_dmas(s.split("|")[0]), _parse_ops(s.split("|")[1])) for s in START]
_ORD1 = _parse_ops("ZZ0 " + " ".join(f"QP{j}" for j in range(U1)))
_ORD2 = _chain(U2, [f"QP{j}" for j in range(P2)] + [f"OP{j}" for j in range(U2)])
_ORD3 = _chain(U3, [f"QP{j}" for j in range(L3)] + [f"OP{j}" for j in range(U3 - NFF)] + [f"FF{U3 - NFF}"])
_ROFF = [sum(ROWS[:t]) for t in range(len(ROWS))]

SEM1 = sum(len(d) for d, _ in _START)
SEMX = SEM1 + N1
SEM2 = SEMX + 1
SEM3 = SEM2 + 2 * N2
SEMO = SEM3 + 2 * N3
NSEM = SEMO + 2 * len(ROWS)


def _kernel(xa, ka, va, wqa, woa, xb, kb, vb, wqb, wob, out_hbm,
            x_buf, wq_s, wq_1, w_2, w_3, k_0, kv, acc, out_buf,
            q_s, q_n, q_l, q_f, p_buf, o_buf, qa_buf, sems):
    c = (DH ** -0.5) * LOG2E
    copy = pltpu.make_async_copy

    def kv_copies(g0, n, sem):
        cps = []
        for which, srcs, lo in ((0, (va, vb), g0), (1, (ka, kb), g0 + 1)):
            slot, g = g0, lo
            while slot < g0 + n:
                br, h = (g // H) % 2, g % H
                m = min(g0 + n - slot, H - h)
                cps.append(copy(srcs[br].at[:, pl.ds(h, m)], kv.at[which, :, pl.ds(slot, m)], sem))
                slot, g = slot + m, g + m
        return cps

    def out_dma(br, t):
        rs = pl.ds(_ROFF[t], ROWS[t])
        return copy(out_buf.at[br, rs, :], out_hbm.at[rs, pl.ds(pl.multiple_of(br * D, D), D)],
                    sems.at[SEMO + br * len(ROWS) + t])

    def src(g):
        return ((wqa, woa), (wqb, wob))[g // H] + ((g % H) * DH,)

    def start_copies():
        cps, si = [], 0
        for dl, _ in _START:
            seg = []
            for kind, (lo, hi), (k0, k1) in dl:
                cs = pl.ds(lo * 128, (hi - lo) * 128)
                if kind == "x":
                    seg.append(copy(xa.at[:, cs], x_buf.at[0, :, cs], sems.at[si]))
                elif kind == "q":
                    rs = pl.ds(k0 * 128, (k1 - k0) * 128)
                    seg.append(copy(wqa.at[rs, cs], wq_s.at[rs, cs], sems.at[si]))
                else:
                    seg.append(copy(ka.at[:, 0], k_0, sems.at[si]))
                si += 1
            cps.append(seg)
        return cps

    for seg in start_copies():
        for cp in seg:
            cp.start()
    for i in range(N1):
        if i == 1:
            copy(xb, x_buf.at[1], sems.at[SEMX]).start()
        wq, _, lo = src(S + i * U3)
        copy(wq.at[:, pl.ds(lo, U1 * DH)], wq_1.at[i, :, pl.ds(0, U1 * DH)], sems.at[SEM1 + i]).start()
    for i in range(N2):
        sem = sems.at[SEM2 + 2 * i]
        wq, _, lo = src(S + N1 * U3 + i * P2)
        copy(wq.at[:, pl.ds(lo, P2 * DH)], w_2.at[i, :, pl.ds(D, P2 * DH)], sem).start()
        copy(woa.at[pl.ds(i * D, D), :], w_2.at[i, :, pl.ds(0, D)], sem).start()
        for cp in kv_copies(i * U2, U2, sems.at[SEM2 + 2 * i + 1]):
            cp.start()
    for i in range(N3):
        sem = sems.at[SEM3 + 2 * i]
        wq, wo, lo = src(S + i * U3)
        hw = (L3 // 2) * DH
        for r in range(2):
            copy(wq.at[:, pl.ds(lo + U1 * DH + r * hw, hw)], w_3.at[i, pl.ds(r * D, D), pl.ds(D, hw)], sem).start()
        copy(wo.at[pl.ds(lo, 2 * D), :], w_3.at[i, :, pl.ds(0, D)], sem).start()
        for cp in kv_copies(S + i * U3, U3, sems.at[SEM3 + 2 * i + 1]):
            cp.start()

    def run(order, phase, it):
        colb = lax.broadcasted_iota(jnp.int32, (SQ, 128), 1) // SK
        colh = lax.broadcasted_iota(jnp.int32, (SQ // 2, 128), 1) // SK
        zero = jnp.zeros((SQ // 2, 128), U32)
        br3 = jnp.minimum(it, 1) if phase == 3 else None
        pbr = {0: 0, 1: it, 2: 1, 3: br3}[phase]
        abr = br3 if phase == 3 else 0
        n_att = {2: U2, 3: U3}.get(phase)
        st = {}

        def u32(a):
            return pltpu.bitcast(a, U32)

        def bf16(a):
            return pltpu.bitcast(a, BF16)

        def sel(i, a, b):
            return bf16(jnp.where(colh == i, u32(a), u32(b)))

        def keep(i, a):
            return bf16(jnp.where(colh != i, zero, u32(a)))

        def drop(i, a):
            return bf16(jnp.where(colh == i, zero, u32(a)))

        def blk(a, i):
            return a[i * SQ:(i + 1) * SQ, :]

        def compact(parts):
            r = parts[GB - 1]
            for i in range(GB - 2, -1, -1):
                r = jnp.where(colb == i, parts[i], r)
            return r

        def wq_cols(j):
            if phase == 1:
                return wq_1[it, :, j * DH:(j + 1) * DH]
            if phase == 2:
                return w_2[it, :, D + j * DH:D + (j + 1) * DH]
            r, jj = divmod(j, L3 // 2)
            return w_3[it, r * D:(r + 1) * D, D + jj * DH:D + (jj + 1) * DH]

        def wo_rows(j, n):
            return (w_2 if phase == 2 else w_3)[it, j * DH:(j + n) * DH, :D]

        def store_q(j, q):
            q = u32(q.astype(BF16))
            if phase == 0:
                if j % U2 == 0:
                    q_f[j // U2] = q
                else:
                    q_s[j] = q
            elif phase == 1:
                if j == 0:
                    q_f[N2 + it] = q
                q_n[it * U1 + j] = q
            elif phase == 2:
                q_n[N1 * U1 + it * P2 + j] = q
            else:
                q_l[j] = q

        def q_next(j, t):
            rs = slice(t * 64, (t + 1) * 64)
            if phase == 2:
                return bf16(q_f[it + 1, rs, :] if j + 1 == U2 else q_s[it * U2 + j + 1, rs, :])
            if j + 1 == U3:
                return bf16(q_n[(br3 + 1) * U1, rs, :])
            if j + 1 >= U1:
                return bf16(q_l[j + 1 - U1, rs, :])
            return bf16(q_n[it * U1 + j + 1, rs, :])

        def kv_tile(which, j, t):
            g0 = it * U2 if phase == 2 else S + it * U3
            return kv[which, t * GB:(t + 1) * GB, g0 + j].reshape(128, DH)

        def softmax(sc):
            mc = compact([jnp.max(jnp.where(colb == i, sc, -jnp.inf), axis=-1, keepdims=True)
                          for i in range(GB)])
            e = jnp.exp2((sc - mc) * c)
            lc = compact([jnp.sum(jnp.where(colb == i, e, 0.0), axis=-1, keepdims=True)
                          for i in range(GB)])
            return (e * pl.reciprocal(lc, approx=False, full_range=False)).astype(BF16)

        for op, j in order:
            if op == "QP":
                store_q(j, jnp.dot(x_buf[pbr], wq_cols(j), preferred_element_type=F32))
            elif op == "QS":
                ja, jb, k0, k1 = j
                q = jnp.dot(x_buf[0, :, k0 * 128:k1 * 128], wq_s[k0 * 128:k1 * 128, ja * DH:jb * DH],
                            preferred_element_type=F32)
                for jj in range(ja, jb):
                    qq = q[:, (jj - ja) * DH:(jj - ja + 1) * DH]
                    if k0 > 0:
                        qq = qa_buf[jj] + qq
                    if k1 == KT:
                        store_q(jj, qq)
                    else:
                        qa_buf[jj] = qq
            elif op == "ZZ":
                acc[it] = jnp.zeros((M, D), F32)
            elif op == "QK":
                for t in range(NG):
                    s = lax.dot_general(bf16(q_f[0, t * 64:(t + 1) * 64, :]),
                                        k_0[t * GB:(t + 1) * GB].reshape(128, DH),
                                        (((1,), (1,)), ((), ())), preferred_element_type=F32)
                    p_buf[t] = u32(softmax(compact([blk(s, i) for i in range(GB)])))
            elif op == "TS":
                for t in range(NG):
                    kt = kv_tile(1, j, t).T
                    q = q_next(j, t)
                    qc = blk(q, GB - 1)
                    for i in range(GB - 2, -1, -1):
                        qc = sel(i, blk(q, i), qc)
                    wdk = jnp.concatenate([keep(i, blk(kt, i)) for i in range(GB)], axis=0)
                    st["ts", t] = (jnp.dot(qc, wdk, preferred_element_type=F32), kt)
            elif op == "MM":
                for t in range(NG):
                    tail_s, kt = st["ts", t]
                    v = kv_tile(0, j, t)
                    q = q_next(j, t)
                    pc = bf16(p_buf[t]) if j == 0 else st["p", t]
                    wdv = jnp.concatenate([keep(i, blk(v, i)) for i in range(GB)], axis=0)
                    tail_o = jnp.dot(pc, wdv, preferred_element_type=F32)
                    mains = []
                    for i in range(GB):
                        w = jnp.concatenate(
                            [drop(i, blk(v, i)) if r == i else keep(i, blk(kt, r)) for r in range(GB)], axis=0)
                        mains.append(jnp.dot(sel(i, pc, blk(q, i)), w, preferred_element_type=F32))
                    pn = softmax(compact(mains) + tail_s)
                    if j + 1 == n_att:
                        p_buf[t] = u32(pn)
                    else:
                        st["p", t] = pn
                    o = jnp.concatenate([jnp.where(colb == i, tail_o, mains[i]) for i in range(GB)], axis=0)
                    o_buf[t * 128:(t + 1) * 128, j * DH:(j + 1) * DH] = o.astype(BF16)
            elif op == "OP":
                acc[abr] = acc[abr] + jnp.dot(o_buf[:, j * DH:(j + 1) * DH], wo_rows(j, 1),
                                              preferred_element_type=F32)
            else:
                for t in range(len(ROWS)):
                    rs = slice(_ROFF[t], _ROFF[t] + ROWS[t])
                    r = acc[abr, rs, :] + jnp.dot(o_buf[rs, j * DH:U3 * DH], wo_rows(j, U3 - j),
                                                  preferred_element_type=F32)
                    acc[abr, rs, :] = r
                    out_buf[abr, rs, :] = r.astype(BF16)

                    @pl.when(it != 1)
                    def _():
                        out_dma(abr, t).start()

    def wait(r, sem):
        copy(r, r, sems.at[sem]).wait()

    def body1(i, carry):
        @pl.when(i == 1)
        def _():
            wait(x_buf.at[1], SEMX)

        wait(wq_1.at[i, :, pl.ds(0, U1 * DH)], SEM1 + i)
        run(_ORD1, 1, i)
        return carry

    def body2(i, carry):
        wait(w_2.at[i, :, pl.ds(0, D + P2 * DH)], SEM2 + 2 * i)
        wait(kv.at[:, :, pl.ds(i * U2, U2)], SEM2 + 2 * i + 1)
        run(_ORD2, 2, i)
        return carry

    def body3(i, carry):
        wait(w_3.at[i, :, pl.ds(0, D + (L3 // 2) * DH)], SEM3 + 2 * i)
        wait(kv.at[:, :, pl.ds(S + i * U3, U3)], SEM3 + 2 * i + 1)
        run(_ORD3, 3, i)
        return carry

    def outer(ph, carry):
        @pl.when(ph == 1)
        def _():
            for seg, (_, ops) in zip(start_copies(), _START):
                for cp in seg:
                    cp.wait()
                run(ops, 0, None)
            lax.fori_loop(0, N1, body1, 0)
            lax.fori_loop(0, N2, body2, 0)
            lax.fori_loop(0, N3, body3, 0)
        return carry

    lax.fori_loop(0, 2, outer, 0)
    for br in range(2):
        for t in range(len(ROWS)):
            out_dma(br, t).wait()


@jax.jit
def pallas_concat_heads__mha_block_cached__mha_block_cached__near_ridge_kernel(
    A_x: jax.Array,
    A_k_cache: jax.Array,
    A_v_cache: jax.Array,
    A_wq: jax.Array,
    A_wo: jax.Array,
    B_x: jax.Array,
    B_k_cache: jax.Array,
    B_v_cache: jax.Array,
    B_wq: jax.Array,
    B_wo: jax.Array,
):
    any_spec = pl.BlockSpec(memory_space=pl.ANY)
    out = pl.pallas_call(
        _kernel,
        in_specs=[any_spec] * 10,
        out_specs=any_spec,
        out_shape=jax.ShapeDtypeStruct((M, 2 * D), BF16),
        scratch_shapes=[
            pltpu.VMEM((2, M, D), BF16),
            pltpu.VMEM((D, S * DH + PAD), BF16),
            pltpu.VMEM((N1, D, W1), BF16),
            pltpu.VMEM((N2, D, W2), BF16),
            pltpu.VMEM((N3, 2 * D, W3), BF16),
            pltpu.VMEM((B, SK, DH), BF16),
            pltpu.VMEM((2, B, 2 * H, SK, DH), BF16),
            pltpu.VMEM((2, M, D), F32),
            pltpu.VMEM((2, M, D), BF16),
            pltpu.VMEM((S, M // 2, DH), U32),
            pltpu.VMEM((N3 * U1, M // 2, DH), U32),
            pltpu.VMEM((L3, M // 2, DH), U32),
            pltpu.VMEM((N2 + N1, M // 2, DH), U32),
            pltpu.VMEM((NG, SQ // 2, 128), U32),
            pltpu.VMEM((M, U3 * DH), BF16),
            pltpu.VMEM((S, M, DH), F32),
            pltpu.SemaphoreType.DMA((NSEM,)),
        ],
        compiler_params=pltpu.CompilerParams(
            vmem_limit_bytes=110 * 1024 * 1024,
            disable_bounds_checks=True,
            disable_semaphore_checks=True,
        ),
    )(A_x.reshape(M, D), A_k_cache, A_v_cache, A_wq, A_wo,
      B_x.reshape(M, D), B_k_cache, B_v_cache, B_wq, B_wo)
    return out.reshape(B, SQ, 2 * D)
```
